```python
import jax
import jax.numpy as jnp

def _softmax(x, axis=-1):
    return jax.nn.softmax(x, axis=axis)

def _gelu(x):
    return jax.nn.gelu(x, approximate=True)

def _silu(x):
    return jax.nn.silu(x)

def _sigmoid(x):
    return jax.nn.sigmoid(x)

def _layernorm(x, axis=-1, eps=1e-05):
    m = jnp.mean(x, axis=axis, keepdims=True)
    v = jnp.var(x, axis=axis, keepdims=True)
    return (x - m) / jnp.sqrt(v + eps)

def _scatter_add(tgt, idx, src, axis=0):
    return tgt.at[idx].add(src)

def _segment_sum(src, seg, n):
    return jax.ops.segment_sum(src, seg, n)

class _Rng:

    def __init__(self, key):
        self._k = key

    def _next(self):
        self._k, sub = jax.random.split(self._k)
        return sub

    def normal(self, shape):
        return jax.random.normal(self._next(), shape, dtype=jnp.bfloat16)

    def randint(self, lo, hi, shape):
        return jax.random.randint(self._next(), shape, lo, hi, dtype=jnp.int32)

    def uniform(self, shape, lo=0.0, hi=1.0):
        return jax.random.uniform(self._next(), shape, jnp.bfloat16, lo, hi)

    def permutation(self, n):
        return jax.random.permutation(self._next(), n)
kernel_name = 'gated_mix__memory_aug_recurrent_mem_tr__ssm_conv_h3__prompt'

def setup_inputs():
    _rng = _Rng(jax.random.key(int.from_bytes(__import__("os").urandom(4), "little")))
    _w = lambda a: (lambda t: t.astype(jnp.bfloat16) if jnp.issubdtype(t.dtype, jnp.floating) else t)(jnp.asarray(a))

    def _A_setup():
        B, S, Dm = (1, 2048, 640)
        H, Dh = (32, 192)
        M, seg = (8, 32)
        seg = min(seg, S)
        S = S // seg * seg
        return {'x': _w((lambda *s: _rng.normal(s) * 0.05)(B, S, Dm)), 'mem0': _w((lambda *s: _rng.normal(s) * 0.05)(B, M, Dm)), 'Wq': _w((lambda *s: _rng.normal(s) * 0.05)(Dm, H, Dh) * Dm ** (-0.5)), 'Wk': _w((lambda *s: _rng.normal(s) * 0.05)(Dm, H, Dh) * Dm ** (-0.5)), 'Wv': _w((lambda *s: _rng.normal(s) * 0.05)(Dm, H, Dh) * Dm ** (-0.5)), 'Wo': _w((lambda *s: _rng.normal(s) * 0.05)(H, Dh, Dm) * (H * Dh) ** (-0.5)), 'seg_len': seg}
    _A_in = _A_setup()

    def _B_setup():
        B, S, D = (1, 2048, 640)
        ks = 4
        return {'q': _w((lambda *s: _rng.normal(s) * 0.05)(B, S, D)), 'k': _w((lambda *s: _rng.normal(s) * 0.05)(B, S, D)), 'v': _w((lambda *s: _rng.normal(s) * 0.05)(B, S, D)), 'shift_k': _w((lambda *s: _rng.normal(s) * 0.05)(D, ks) * 0.5), 'ssm_k': _w((lambda *s: _rng.normal(s) * 0.05)(D, S) * (1.0 / S ** 0.5)), 'ssm_D': _w((lambda *s: _rng.normal(s) * 0.05)(D))}
    _B_in = _B_setup()
    return {'A_x': _A_in['x'], 'A_mem0': _A_in['mem0'], 'A_Wq': _A_in['Wq'], 'A_Wk': _A_in['Wk'], 'A_Wv': _A_in['Wv'], 'A_Wo': _A_in['Wo'], 'A_seg_len': _A_in['seg_len'], 'B_q': _B_in['q'], 'B_k': _B_in['k'], 'B_v': _B_in['v'], 'B_shift_k': _B_in['shift_k'], 'B_ssm_k': _B_in['ssm_k'], 'B_ssm_D': _B_in['ssm_D'], 'gate_w': _w((lambda *s: _rng.normal(s) * 0.05)(640))}

def reference(A_x, A_mem0, A_Wq, A_Wk, A_Wv, A_Wo, A_seg_len, B_q, B_k, B_v, B_shift_k, B_ssm_k, B_ssm_D, gate_w):

    def _A_ref(x, mem0, Wq, Wk, Wv, Wo, seg_len):
        B, S, Dm = x.shape
        H, Dh = (Wq.shape[1], Wq.shape[2])
        M = mem0.shape[1]
        scale = Dh ** (-0.5)
        n_seg = S // seg_len
        L = M + seg_len
        idx = jnp.arange(L)
        mask = (idx[:, None] < M) | (idx[:, None] >= idx[None, :])
        mem = mem0
        outs = []
        for s in range(n_seg):
            xs = x[:, s * seg_len:(s + 1) * seg_len, :].copy()
            h = jnp.concatenate([mem, xs], axis=1)
            q = jnp.einsum('btd,dhe->bhte', h, Wq)
            k = jnp.einsum('btd,dhe->bhte', h, Wk)
            v = jnp.einsum('btd,dhe->bhte', h, Wv)
            scores = jnp.einsum('bhqe,bhke->bhqk', q, k) * scale
            scores = jnp.where(mask[None, None], scores, -1000000000.0)
            p = _softmax(scores, axis=-1)
            o = jnp.einsum('bhqk,bhke->bhqe', p, v)
            o = jnp.einsum('bhte,hed->btd', o, Wo)
            mem = o[:, :M, :].copy()
            outs.append(o[:, M:, :])
        return jnp.concatenate(outs, axis=1)

    def _B_ref(q, k, v, shift_k, ssm_k, ssm_D):
        B, S, D = q.shape
        ks = shift_k.shape[-1]
        k_pad = jnp.pad(k, ((0, 0), (ks - 1, 0), (0, 0)))
        k_shift = jnp.zeros_like(k)
        for t in range(ks):
            k_shift = k_shift + k_pad[:, t:t + S, :] * shift_k[:, ks - 1 - t][None, None, :]
        kv = k_shift * v
        L = 2 * S
        kv_pad = jnp.pad(kv, ((0, 0), (0, S), (0, 0)))
        kf_pad = jnp.pad(ssm_k, ((0, 0), (0, S)))
        kv_f = (lambda x, axes=(-2, -1): jnp.fft.rfft2(x.astype(jnp.float32), axes=axes))(kv_pad[:, None, :, :], axes=(1, 2))
        kf_f = (lambda x, axes=(-2, -1): jnp.fft.rfft2(x.astype(jnp.float32), axes=axes))(kf_pad[:, None, :], axes=(1, 2))
        kf_f = (lambda x, *d: x.transpose(*d))(kf_f, 1, 2, 0)
        y_f = kv_f * kf_f[None, :, :, :]
        y = (lambda x, s, axes=(-2, -1): jnp.fft.irfft2(x, s=s, axes=axes).astype(jnp.bfloat16))(y_f, (1, L), axes=(1, 2))[:, 0, :S, :]
        y = y + kv * ssm_D[None, None, :]
        return q * y
    x = A_x
    g = _sigmoid((x * gate_w).sum(-1, keepdims=True))
    a = _A_ref(x, A_mem0, A_Wq, A_Wk, A_Wv, A_Wo, A_seg_len)
    b = _B_ref(x, B_k, B_v, B_shift_k, B_ssm_k, B_ssm_D)
    return g * a + (1 - g) * b
```

```python
import functools

import jax
import jax.numpy as jnp
import numpy as np
from jax import lax
from jax.experimental import pallas as pl
from jax.experimental.pallas import tpu as pltpu

f32 = jnp.float32
bf16 = jnp.bfloat16
NN = (((1,), (0,)), ((), ()))
NT = (((1,), (1,)), ((), ()))
LANES = 128
T = 128


def _dft_matrices():
    theta = 2.0 * np.pi * (np.arange(T, dtype=np.float64) + 0.5) / (2 * T)
    ang = theta[:, None] * np.arange(T, dtype=np.float64)[None, :]
    fwd = np.concatenate([np.cos(ang), -np.sin(ang)], axis=0)
    inv = fwd.T / T
    return fwd.astype(np.float32), inv.astype(np.float32)


def _kernel(
    x_hbm, mem0_ref, wq_hbm, wk_hbm, wv_hbm, wo_hbm, bk_hbm, bv_hbm, shift_ref,
    ssmk_hbm, ssmd_ref, gw_ref, fwd_ref, inv_ref,
    o_ref,
    x_ref, bk_ref, bv_ref, ssmk_ref, wraw_ref, w_ref, wo_ref, kv_ref, xf_ref,
    cf_ref, yf_ref, bt_ref, g_ref, h_ref, att_ref, sems,
    *, S, D, H, Dh, M, seg, segs_per_step,
):
    L = M + seg
    n_pairs = H // 2
    tpp = 2 * Dh // LANES
    n_col = D // LANES
    n_chunk = S // T
    pid = pl.program_id(0)

    @pl.when(pid == 0)
    def _prologue():
        cps = [
            pltpu.make_async_copy(bk_hbm, bk_ref, sems.at[0]),
            pltpu.make_async_copy(bv_hbm, bv_ref, sems.at[1]),
            pltpu.make_async_copy(ssmk_hbm, ssmk_ref, sems.at[2]),
            pltpu.make_async_copy(x_hbm, x_ref, sems.at[3]),
            pltpu.make_async_copy(wq_hbm, wraw_ref.at[0], sems.at[4]),
            pltpu.make_async_copy(wk_hbm, wraw_ref.at[1], sems.at[5]),
            pltpu.make_async_copy(wv_hbm, wraw_ref.at[2], sems.at[6]),
            pltpu.make_async_copy(wo_hbm, wo_ref, sems.at[7]),
        ]
        for cp in cps:
            cp.start()

        cps[0].wait()
        cps[1].wait()
        shift = shift_ref[...].astype(f32)
        n_shift = shift.shape[0]

        def kv_chunk(a, c):
            r0 = pl.multiple_of(a * T, T)
            rp = pl.multiple_of(jnp.maximum(r0 - 16, 0), 16)
            prev = bk_ref[pl.ds(rp, 16), :].astype(f32)[8:16]
            prev = jnp.where(a > 0, prev, 0.0)
            ext = jnp.concatenate([prev, bk_ref[pl.ds(r0, T), :].astype(f32)], axis=0)
            acc = ext[8:8 + T] * shift[0:1]
            for j in range(1, n_shift):
                acc = acc + ext[8 - j:8 - j + T] * shift[j:j + 1]
            kv = acc * bv_ref[pl.ds(r0, T), :].astype(f32)
            kv_ref[pl.ds(r0, T), :] = kv.astype(bf16)
            return c

        lax.fori_loop(0, n_chunk, kv_chunk, 0)

        cps[3].wait()
        gw = gw_ref[...].astype(f32)

        def gate_chunk(a, c):
            r0 = pl.multiple_of(a * T, T)
            z = jnp.sum(x_ref[pl.ds(r0, T), :].astype(f32) * gw, axis=1, keepdims=True)
            g_ref[pl.ds(r0, T), :] = jnp.broadcast_to(jax.nn.sigmoid(z), (T, LANES))
            return c

        lax.fori_loop(0, n_chunk, gate_chunk, 0)

        cps[2].wait()
        sgn = jnp.where(
            (lax.broadcasted_iota(jnp.int32, (T, LANES), 0) & 1) == 0, 1.0, -1.0
        ).astype(f32)

        for cg in range(n_col):
            cs = slice(cg * LANES, (cg + 1) * LANES)

            def fwd_x(a, c, cs=cs):
                r0 = pl.multiple_of(a * T, T)
                xf_ref[a] = jnp.dot(fwd_ref[...], kv_ref[pl.ds(r0, T), cs],
                                    preferred_element_type=f32)
                return c

            lax.fori_loop(0, n_chunk, fwd_x, 0, unroll=4)

            prev = None
            for dl in range(n_chunk):
                kf = lax.dot_general(fwd_ref[...], ssmk_ref[cs, dl * T:(dl + 1) * T], NT,
                                     preferred_element_type=f32)
                if prev is None:
                    cf_ref[dl] = kf
                else:
                    cf_ref[dl, 0:T, :] = kf[0:T] - sgn * prev[T:2 * T]
                    cf_ref[dl, T:2 * T, :] = kf[T:2 * T] + sgn * prev[0:T]
                prev = kf

            def freq_tile(ft, c):
                f0 = pl.multiple_of(ft * 8, 8)
                re, im = pl.ds(f0, 8), pl.ds(T + f0, 8)
                cr = [cf_ref[dl, re, :] for dl in range(n_chunk)]
                ci = [cf_ref[dl, im, :] for dl in range(n_chunk)]
                for a in range(n_chunk):
                    yr = yi = None
                    for dl in range(a + 1):
                        xr = xf_ref[a - dl, re, :]
                        xi = xf_ref[a - dl, im, :]
                        tr = cr[dl] * xr - ci[dl] * xi
                        ti = cr[dl] * xi + ci[dl] * xr
                        yr = tr if yr is None else yr + tr
                        yi = ti if yi is None else yi + ti
                    yf_ref[a, re, :] = yr
                    yf_ref[a, im, :] = yi
                return c

            lax.fori_loop(0, T // 8, freq_tile, 0)

            dvec = ssmd_ref[:, cs].astype(f32)

            def inv_y(a, c, cs=cs, dvec=dvec):
                r0 = pl.multiple_of(a * T, T)
                rows = pl.ds(r0, T)
                y = jnp.dot(inv_ref[...], yf_ref[a].astype(bf16), preferred_element_type=f32)
                y = y + kv_ref[rows, cs].astype(f32) * dvec
                b = x_ref[rows, cs].astype(f32) * y
                bt_ref[rows, cs] = (1.0 - g_ref[rows, :]) * b
                return c

            lax.fori_loop(0, n_chunk, inv_y, 0, unroll=4)

        for m in range(3):
            cps[4 + m].wait()

            def tr(p, c, m=m):
                for t in range(tpp):
                    r0 = pl.multiple_of((p * tpp + t) * LANES, LANES)
                    w_ref[(p * 3 + m) * tpp + t] = wraw_ref[m, pl.ds(r0, LANES), :].T
                return c

            lax.fori_loop(0, n_pairs, tr, 0)
        cps[7].wait()
        h_ref[0:M, :] = mem0_ref[...].astype(f32)

    def step(si, carry):
        r_loc = pl.multiple_of(si * seg, seg)
        r_glb = pl.multiple_of((pid * segs_per_step + si) * seg, seg)
        h_ref[M:L, :] = x_ref[pl.ds(r_glb, seg), :].astype(f32)

        half = LANES // 2
        row = lax.broadcasted_iota(jnp.int32, (L, LANES), 0)
        lane = lax.broadcasted_iota(jnp.int32, (L, LANES), 1)
        key = lane & (half - 1)
        is_key = key < L
        allowed = (row < M) | (row >= key)
        first = lane < half
        zpad = jnp.zeros((half - L, LANES), f32)
        zrows = jnp.zeros((L, LANES), f32)

        def proj(p, m):
            return [
                jnp.dot(h_ref[...], w_ref[(p * 3 + m) * tpp + t], preferred_element_type=f32)
                for t in range(tpp)
            ]

        def blockdiag(t3):
            a, mid, b = t3
            return (
                jnp.concatenate([a, zpad, zrows, zpad], axis=0).astype(bf16),
                jnp.concatenate([jnp.where(first, mid, 0.0), zpad,
                                 jnp.where(first, 0.0, mid), zpad], axis=0).astype(bf16),
                jnp.concatenate([zrows, zpad, b, zpad], axis=0).astype(bf16),
            )

        def scores(q, k):
            kb = blockdiag(k)
            acc = None
            for t in range(tpp):
                y = lax.dot_general(q[t], kb[t], NT, preferred_element_type=f32)
                acc = y if acc is None else acc + y
            return acc

        def softmax(sc):
            sc = jnp.where(allowed, sc * (Dh ** -0.5), -1000000000.0)
            ninf = -jnp.inf
            m0 = jnp.max(jnp.where(first & is_key, sc, ninf), axis=1, keepdims=True)
            m1 = jnp.max(jnp.where(is_key & ~first, sc, ninf), axis=1, keepdims=True)
            e = jnp.exp(jnp.where(is_key, sc - jnp.where(first, m0, m1), ninf))
            s0 = jnp.sum(jnp.where(first, e, 0.0), axis=1, keepdims=True)
            s1 = jnp.sum(jnp.where(first, 0.0, e), axis=1, keepdims=True)
            return e / jnp.where(first, s0, s1)

        def attend(prob, v, p):
            vb = blockdiag(v)
            for t in range(tpp):
                c0 = (p * tpp + t) * LANES
                att_ref[:, c0:c0 + LANES] = jnp.dot(prob, vb[t], preferred_element_type=f32)

        lag1, lag2 = 1, 3
        q, k, v, sc = {}, {}, {}, {}
        for i in range(n_pairs + lag2):
            if i < n_pairs:
                k[i] = proj(i, 1)
                q[i] = proj(i, 0)
                v[i] = proj(i, 2)
            if 0 <= i - lag1 < n_pairs:
                sc[i - lag1] = scores(q[i - lag1], k[i - lag1])
            if 0 <= i - lag2 < n_pairs:
                attend(softmax(sc[i - lag2]), v[i - lag2], i - lag2)

        n_kc = 2
        kc = H * Dh // n_kc
        accs = [None] * n_col
        for ch in range(n_kc):
            for n in range(n_col):
                y = jnp.dot(att_ref[:, ch * kc:(ch + 1) * kc],
                            wo_ref[ch * kc:(ch + 1) * kc, n * LANES:(n + 1) * LANES],
                            preferred_element_type=f32)
                accs[n] = y if accs[n] is None else accs[n] + y
        gate = g_ref[pl.ds(r_glb, seg), :]
        for n in range(n_col):
            cs = slice(n * LANES, (n + 1) * LANES)
            h_ref[0:M, cs] = accs[n][0:M]
            res = gate * accs[n][M:L] + bt_ref[pl.ds(r_glb, seg), cs]
            o_ref[pl.ds(r_loc, seg), cs] = res.astype(o_ref.dtype)
        return carry

    lax.fori_loop(0, segs_per_step, step, 0)


@functools.partial(jax.jit, static_argnames=("A_seg_len",))
def pallas_gated_mix__memory_aug_recurrent_mem_tr__ssm_conv_h3__prompt_kernel(
    A_x: jax.Array,
    A_mem0: jax.Array,
    A_Wq: jax.Array,
    A_Wk: jax.Array,
    A_Wv: jax.Array,
    A_Wo: jax.Array,
    A_seg_len: int,
    B_q: jax.Array,
    B_k: jax.Array,
    B_v: jax.Array,
    B_shift_k: jax.Array,
    B_ssm_k: jax.Array,
    B_ssm_D: jax.Array,
    gate_w: jax.Array,
):
    del B_q
    B, S, D = A_x.shape
    H, Dh = A_Wq.shape[1], A_Wq.shape[2]
    M = A_mem0.shape[1]
    seg = int(A_seg_len)
    n_seg = S // seg
    assert B == 1 and S % T == 0 and D % LANES == 0 and H % 2 == 0
    assert 2 * Dh == 3 * LANES and M % 8 == 0 and seg % 16 == 0 and M + seg <= LANES // 2
    segs_per_step = 8
    assert n_seg % segs_per_step == 0
    E = H * Dh
    n_chunk = S // T

    def head_major(w):
        return jnp.transpose(w, (1, 2, 0)).reshape(E, D)

    fwd, inv = _dft_matrices()
    hbm = pl.BlockSpec(memory_space=pl.ANY)

    def full(shape):
        return pl.BlockSpec(shape, lambda i: (0,) * len(shape))

    ks = B_shift_k.shape[1]
    out = pl.pallas_call(
        functools.partial(_kernel, S=S, D=D, H=H, Dh=Dh, M=M, seg=seg,
                          segs_per_step=segs_per_step),
        grid=(n_seg // segs_per_step,),
        in_specs=[
            hbm, full((M, D)), hbm, hbm, hbm, hbm, hbm, hbm, full((ks, D)),
            hbm, full((1, D)), full((1, D)), full((2 * T, T)), full((T, 2 * T)),
        ],
        out_specs=pl.BlockSpec((segs_per_step * seg, D), lambda i: (i, 0)),
        out_shape=jax.ShapeDtypeStruct((S, D), A_x.dtype),
        scratch_shapes=[
            pltpu.VMEM((S, D), bf16),
            pltpu.VMEM((S, D), bf16),
            pltpu.VMEM((S, D), bf16),
            pltpu.VMEM((D, S), bf16),
            pltpu.VMEM((3, E, D), bf16),
            pltpu.VMEM((3 * E // LANES, D, LANES), bf16),
            pltpu.VMEM((E, D), bf16),
            pltpu.VMEM((S, D), bf16),
            pltpu.VMEM((n_chunk, 2 * T, LANES), f32),
            pltpu.VMEM((n_chunk, 2 * T, LANES), f32),
            pltpu.VMEM((n_chunk, 2 * T, LANES), f32),
            pltpu.VMEM((S, D), f32),
            pltpu.VMEM((S, LANES), f32),
            pltpu.VMEM((M + seg, D), f32),
            pltpu.VMEM((M + seg, E), f32),
            pltpu.SemaphoreType.DMA((8,)),
        ],
        compiler_params=pltpu.CompilerParams(
            dimension_semantics=("arbitrary",),
            vmem_limit_bytes=110 * 1024 * 1024,
        ),
    )(
        A_x.reshape(S, D), A_mem0.reshape(M, D),
        head_major(A_Wq), head_major(A_Wk), head_major(A_Wv), A_Wo.reshape(E, D),
        B_k.reshape(S, D), B_v.reshape(S, D), B_shift_k.T, B_ssm_k,
        B_ssm_D.reshape(1, D), gate_w.reshape(1, D),
        jnp.asarray(fwd, dtype=bf16), jnp.asarray(inv, dtype=bf16),
    )
    return out.reshape(B, S, D)
```

```python
import functools

import jax
import jax.numpy as jnp
import numpy as np
from jax import lax
from jax.experimental import pallas as pl
from jax.experimental.pallas import tpu as pltpu

f32 = jnp.float32
u32 = jnp.uint32
bf16 = jnp.bfloat16
NT = (((1,), (1,)), ((), ()))
LANES = 128
T = 128
N_STAGE = 3


def _dft_matrices(blk):
    theta = 2.0 * np.pi * (np.arange(T, dtype=np.float64) + 0.5) / (2 * T)
    ang = theta[:, None] * np.arange(T, dtype=np.float64)[None, :]
    fwd = np.stack([np.cos(ang).reshape(-1, blk, T), -np.sin(ang).reshape(-1, blk, T)], axis=1).reshape(2 * T, T)
    inv = fwd.T / T
    return fwd.astype(np.float32), inv.astype(np.float32)


def _kernel(
    x_hbm, mem0_ref, wq_hbm, wk_hbm, wv_hbm, wo_hbm, bk_hbm, bv_hbm, shift_ref,
    ssmk_hbm, ssmd_ref, gw_ref, fwd_ref, inv_ref,
    o_ref,
    x_ref, bk_ref, bv_ref, ssmk_ref, stage_ref, w_ref, wo_ref, xh_ref, q_ring, k_ring, v_ring,
    kv_ref, xf_ref, cf_ref, yf_ref, kprev_ref, mem_ref, att_ref,
    x_sem, w_sem, c_sem,
    *, S, D, H, Dh, M, seg, segs_per_step, ahead, ring_rows, ring_off,
):
    L = M + seg
    n_pairs = H // 2
    pw = 2 * Dh
    tpp = pw // LANES
    n_col = D // LANES
    n_chunk = S // T
    per = T // seg
    tok = seg - M
    rings = (q_ring, k_ring, v_ring)
    w_hbm = (wq_hbm, wk_hbm, wv_hbm, wo_hbm)
    pid = pl.program_id(0)

    def lanes(i):
        return slice(i * LANES, (i + 1) * LANES)

    def weight_copies(a):
        wrows = pl.ds(pl.multiple_of(a * pw, pw), pw)
        return [pltpu.make_async_copy(w_hbm[m].at[wrows, :], stage_ref.at[a % N_STAGE, m], w_sem.at[m, a])
                for m in range(4)]

    def conv_copies(a):
        trows = pl.ds(pl.multiple_of(a * T, T), T)
        return [
            pltpu.make_async_copy(bk_hbm.at[trows, :], bk_ref.at[trows, :], c_sem.at[0, a]),
            pltpu.make_async_copy(bv_hbm.at[trows, :], bv_ref.at[trows, :], c_sem.at[1, a]),
            pltpu.make_async_copy(ssmk_hbm.at[:, trows], ssmk_ref.at[a], c_sem.at[2, a]),
        ]

    @pl.when(pid == 0)
    def _prologue():
        x_head = pltpu.make_async_copy(x_hbm.at[0:ahead, :], x_ref.at[0:ahead, :], x_sem.at[0])
        x_tail = pltpu.make_async_copy(x_hbm.at[ahead:S, :], x_ref.at[ahead:S, :], x_sem.at[1])
        x_head.start()
        for a in range(N_STAGE - 1):
            for cp in weight_copies(a) + conv_copies(a):
                cp.start()

        def zero(a, c):
            for q in range(per):
                xf_ref[q, a] = jnp.zeros(xf_ref.shape[2:], f32)
            return c

        lax.fori_loop(0, n_chunk - 1, zero, 0)
        kprev_ref[...] = jnp.zeros(kprev_ref.shape, f32)
        mem_ref[...] = mem0_ref[...].astype(f32)

        def forward_k(a):
            sgn = jnp.where((lax.broadcasted_iota(jnp.int32, (seg, LANES), 0) & 1) == 0, 1.0, -1.0)
            for cg in range(n_col):
                cs = lanes(cg)
                kf = lax.dot_general(fwd_ref[...], ssmk_ref[a, cs, :], NT, preferred_element_type=f32)
                for q in range(per):
                    re, im = slice(2 * q * seg, (2 * q + 1) * seg), slice((2 * q + 1) * seg, (2 * q + 2) * seg)
                    cf_ref[q, a, 0:seg, cs] = kf[re] - sgn * kprev_ref[im, cs]
                    cf_ref[q, a, seg:2 * seg, cs] = kf[im] + sgn * kprev_ref[re, cs]
                kprev_ref[:, cs] = kf

        def forward_x(a):
            r0 = pl.multiple_of(a * T, T)
            rows = pl.ds(r0, T)
            rp = pl.ds(pl.multiple_of(jnp.maximum(r0 - 16, 0), 16), 16)
            for cg in range(n_col):
                cs = lanes(cg)
                shift = shift_ref[:, cs].astype(f32)
                prev = jnp.where(a > 0, bk_ref[rp, cs].astype(f32)[8:16], 0.0)
                ext = jnp.concatenate([prev, bk_ref[rows, cs].astype(f32)], axis=0)
                ksh = ext[8:8 + T] * shift[0:1]
                for j in range(1, shift.shape[0]):
                    ksh = ksh + ext[8 - j:8 - j + T] * shift[j:j + 1]
                kv = (ksh * bv_ref[rows, cs].astype(f32)).astype(bf16)
                kv_ref[rows, cs] = kv
                xf = jnp.dot(fwd_ref[...], kv, preferred_element_type=f32)
                for q in range(per):
                    xf_ref[q, a + n_chunk - 1, :, cs] = xf[2 * q * seg:(2 * q + 2) * seg]

        x_head.wait()
        xh_ref[...] = pltpu.bitcast(x_ref[0:ahead, :], u32)

        def chunk(a, c):
            @pl.when(a + N_STAGE - 1 < n_chunk)
            def _():
                for cp in weight_copies(a + N_STAGE - 1) + conv_copies(a + N_STAGE - 1):
                    cp.start()

            @pl.when(a == n_chunk - N_STAGE + 1)
            def _():
                x_tail.start()

            for cp in weight_copies(a) + conv_copies(a):
                cp.wait()

            slot = a % N_STAGE
            wo_ref[pl.ds(pl.multiple_of(a * (pw // 2), pw // 2), pw // 2), :] = pltpu.bitcast(
                stage_ref[slot, 3], u32)
            n_blk = 3 * tpp
            mb = 512
            nrb = ahead // mb
            for blk in range(n_blk):
                m, t = divmod(blk, tpp)
                raw = stage_ref[slot, m, lanes(t), :]
                w_ref[a * n_blk + blk] = pltpu.bitcast(raw.T, u32)
                for rb in range(nrb):
                    xh = pltpu.bitcast(xh_ref[rb * mb // 2:(rb + 1) * mb // 2, :], bf16)
                    y = lax.dot_general(xh, raw, NT, preferred_element_type=f32)
                    rings[m][a * tpp + t, ring_off + rb * mb:ring_off + (rb + 1) * mb, :] = y.astype(bf16)
                if blk == 1:
                    forward_k(a)
                if blk == 4:
                    forward_x(a)
            return c

        lax.fori_loop(0, n_chunk, chunk, 0)
        for q in range(per):
            cr, ci = cf_ref[q, 0, 0:seg], cf_ref[q, 0, seg:2 * seg]
            xr, xi = xf_ref[q, n_chunk - 1, 0:seg], xf_ref[q, n_chunk - 1, seg:2 * seg]
            xf_ref[q, 2 * n_chunk - 1, 0:seg] = cr * xr - ci * xi
            xf_ref[q, 2 * n_chunk - 1, seg:2 * seg] = cr * xi + ci * xr
        x_tail.wait()

    def step(si, carry):
        s = pid * segs_per_step + si
        r_loc = pl.multiple_of(si * seg, seg)
        r_glb = pl.multiple_of(s * seg, seg)
        rd = pl.ds(pl.multiple_of(lax.rem(s * seg + ring_off, ring_rows), seg), seg)
        wr = pl.ds(pl.multiple_of(lax.rem(s * tok, ring_rows), 8), tok)
        x_new = x_ref[pl.ds(pl.multiple_of(ahead + s * tok, 8), tok), :]
        lhs = jnp.concatenate([mem_ref[...], x_new.astype(f32)], axis=0).astype(bf16)

        half = LANES // 2
        row = lax.broadcasted_iota(jnp.int32, (L, LANES), 0)
        lane = lax.broadcasted_iota(jnp.int32, (L, LANES), 1)
        key = lane & (half - 1)
        is_key = key < L
        allowed = (row < M) | (key >= seg) | (row - M >= key)
        first = lane < half
        first_k = lax.broadcasted_iota(jnp.int32, (half, LANES), 1) < half
        zhalf = jnp.zeros((half, LANES), bf16)
        row_first = lax.broadcasted_iota(jnp.int32, (LANES, LANES), 0) < half
        col_first = lax.broadcasted_iota(jnp.int32, (LANES, LANES), 1) < half

        def proj(p, m):
            out = []
            for t in range(tpp):
                y = jnp.dot(lhs, pltpu.bitcast(w_ref[(p * 3 + m) * tpp + t], bf16), preferred_element_type=f32)
                rings[m][p * tpp + t, wr, :] = y[M:].astype(bf16)
                out.append(y[0:M])
            return out

        def load(p, m):
            return [rings[m][p * tpp + t, rd, :] for t in range(tpp)]

        def keys(tok3, mem3):
            return [
                jnp.concatenate(
                    [tk, jnp.concatenate([mm, jnp.zeros((half - L, LANES), f32)], axis=0).astype(bf16)],
                    axis=0)
                for tk, mm in zip(tok3, mem3)]

        def blockdiag(tok3, mem3):
            a, mid, b = keys(tok3, mem3)
            zero = jnp.zeros_like(mid)
            return (
                jnp.concatenate([a, zhalf], axis=0),
                jnp.concatenate([jnp.where(first_k, mid, zero), jnp.where(first_k, zero, mid)], axis=0),
                jnp.concatenate([zhalf, b], axis=0),
            )

        def keys_t(k_tok, k_mem):
            a, mid, b = keys(k_tok, k_mem)
            outer = jnp.concatenate([a, b], axis=0).T
            inner = jnp.concatenate([mid, mid], axis=0).T
            return outer, inner

        def scores(q_tok, q_mem, kt):
            outer, inner = kt
            zero = jnp.zeros_like(outer)
            kb = (jnp.where(col_first, outer, zero), jnp.where(col_first == row_first, inner, zero),
                  jnp.where(col_first, zero, outer))
            acc = None
            for t in range(tpp):
                q = jnp.concatenate([q_mem[t], q_tok[t].astype(f32)], axis=0)
                y = jnp.dot(q, kb[t], preferred_element_type=f32)
                acc = y if acc is None else acc + y
            return acc

        def softmax(sc):
            sc = jnp.where(allowed, sc * (Dh ** -0.5), -1000000000.0)
            ninf = -jnp.inf
            m0 = jnp.max(jnp.where(first & is_key, sc, ninf), axis=1, keepdims=True)
            m1 = jnp.max(jnp.where(is_key & ~first, sc, ninf), axis=1, keepdims=True)
            e = jnp.exp(jnp.where(is_key, sc - jnp.where(first, m0, m1), ninf))
            s0 = jnp.sum(jnp.where(first, e, 0.0), axis=1, keepdims=True)
            s1 = jnp.sum(jnp.where(first, 0.0, e), axis=1, keepdims=True)
            return e / jnp.where(first, s0, s1)

        def attend(prob, v_tok, v_mem, p):
            vb = blockdiag(v_tok, v_mem)
            for t in range(tpp):
                att_ref[:, lanes(p * tpp + t)] = jnp.dot(prob, vb[t], preferred_element_type=f32)

        chunk_id, part = s // per, s % per
        nxt = jnp.minimum(chunk_id + 1, n_chunk - 1)
        c_now = cf_ref.at[part]
        x_now = xf_ref.at[part, pl.ds(nxt, n_chunk)]
        y_now = xf_ref.at[part, 2 * n_chunk - 1 + (chunk_id + 1) % 2]

        def mac(ft, cg):
            re, im, cs = slice(ft * 8, ft * 8 + 8), slice(seg + ft * 8, seg + ft * 8 + 8), lanes(cg)
            yr = yi = None
            for dl in range(n_chunk):
                cr, ci = c_now[dl, re, cs], c_now[dl, im, cs]
                xr, xi = x_now[n_chunk - 1 - dl, re, cs], x_now[n_chunk - 1 - dl, im, cs]
                tr = cr * xr - ci * xi
                ti = cr * xi + ci * xr
                yr = tr if yr is None else yr + tr
                yi = ti if yi is None else yi + ti
                if (dl + 1) % 2 == 0 and dl + 1 < n_chunk:
                    y_now[im, cs] = yi
            y_now[re, cs] = yr
            y_now[im, cs] = yi

        def branch_b():
            rows = pl.ds(r_glb, seg)
            inv = inv_ref[pl.ds(pl.multiple_of(part * seg, seg), seg), :]
            x = x_ref[rows, :].astype(f32)
            z = jnp.sum(x * gw_ref[...].astype(f32), axis=1, keepdims=True)
            gate = jnp.broadcast_to(jax.nn.sigmoid(z), (seg, LANES))
            out = []
            for cg in range(n_col):
                cs = lanes(cg)
                y = jnp.dot(inv, xf_ref[:, 2 * n_chunk - 1 + chunk_id % 2, :, cs].reshape(2 * T, LANES).astype(bf16), preferred_element_type=f32)
                y = y + kv_ref[rows, cs].astype(f32) * ssmd_ref[:, cs].astype(f32)
                out.append((1.0 - gate) * (x[:, cs] * y))
            return gate, out

        todo = [(ft, cg) for cg in range(n_col) for ft in range(seg // 8)]
        mac_lo, mac_hi = 10, 58
        accs = [None] * n_col

        def out_proj(p0, p1):
            for n in range(n_col):
                y = jnp.dot(att_ref[:, p0 * pw:p1 * pw], pltpu.bitcast(wo_ref[p0 * pw // 2:p1 * pw // 2, lanes(n)], bf16),
                            preferred_element_type=f32)
                accs[n] = y if accs[n] is None else accs[n] + y

        d_kt, d_sc, d_sm, d_pv = 3, 7, 9, 13
        woc = 1
        qm, km, vm, kt, sc, pr = {}, {}, {}, {}, {}, {}
        done = 0

        def due(u, d):
            p, r = divmod(u - d, 3)
            return p if r == 0 and 0 <= p < n_pairs else None

        for u in range(3 * n_pairs + d_pv - 2):
            p_kt, p_sc, p_sm, p_pv = due(u, d_kt), due(u, d_sc), due(u, d_sm), due(u, d_pv)
            if p_kt is not None:
                k_tok = load(p_kt, 1)
            if p_sc is not None:
                q_tok = load(p_sc, 0)
            if p_pv is not None:
                v_tok = load(p_pv, 2)
            i, r = divmod(u, 3)
            if i < n_pairs:
                (km, qm, vm)[r][i] = proj(i, (1, 0, 2)[r])
            else:
                out_proj(done, done + woc)
                done += woc
            if p_sc is not None:
                sc[p_sc] = scores(q_tok, qm[p_sc], kt[p_sc])
            if p_pv is not None:
                attend(pr[p_pv], v_tok, vm[p_pv], p_pv)
            if p_kt is not None:
                kt[p_kt] = keys_t(k_tok, km[p_kt])
            if p_sm is not None:
                pr[p_sm] = softmax(sc[p_sm])
            if u == 3:
                gate, bt = branch_b()
            if mac_lo <= u < mac_hi and not 0:
                n = len(todo)
                for ft, cg in todo[(u - mac_lo) * n // (mac_hi - mac_lo):(u + 1 - mac_lo) * n // (mac_hi - mac_lo)]:
                    mac(ft, cg)
        out_proj(done, n_pairs)

        for n in range(n_col):
            cs = lanes(n)
            mem_ref[:, cs] = accs[n][0:M]
            res = gate * accs[n][M:L] + bt[n]
            o_ref[pl.ds(r_loc, seg), cs] = res.astype(o_ref.dtype)
        return carry

    lax.fori_loop(0, segs_per_step, step, 0)


@functools.partial(jax.jit, static_argnames=("A_seg_len",))
def pallas_gated_mix__memory_aug_recurrent_mem_tr__ssm_conv_h3__prompt_kernel(
    A_x: jax.Array,
    A_mem0: jax.Array,
    A_Wq: jax.Array,
    A_Wk: jax.Array,
    A_Wv: jax.Array,
    A_Wo: jax.Array,
    A_seg_len: int,
    B_q: jax.Array,
    B_k: jax.Array,
    B_v: jax.Array,
    B_shift_k: jax.Array,
    B_ssm_k: jax.Array,
    B_ssm_D: jax.Array,
    gate_w: jax.Array,
):
    del B_q
    B, S, D = A_x.shape
    H, Dh = A_Wq.shape[1], A_Wq.shape[2]
    M = A_mem0.shape[1]
    seg = int(A_seg_len)
    n_seg = S // seg
    E = H * Dh
    n_chunk = S // T
    segs_per_step = 8
    ahead = n_seg * M
    ring_rows, ring_off = 576, 64
    assert (B, S, M, seg, H // 2, 2 * Dh) == (1, 2048, 8, 32, n_chunk, 3 * LANES) and D % LANES == 0

    def head_major(w):
        return jnp.transpose(w, (1, 2, 0)).reshape(E, D)

    fwd, inv = _dft_matrices(seg)
    hbm = pl.BlockSpec(memory_space=pl.ANY)

    def full(shape):
        return pl.BlockSpec(shape, lambda i: (0,) * len(shape))

    ks = B_shift_k.shape[1]
    ring = pltpu.VMEM((E // LANES, ring_rows, LANES), bf16)
    out = pl.pallas_call(
        functools.partial(_kernel, S=S, D=D, H=H, Dh=Dh, M=M, seg=seg,
                          segs_per_step=segs_per_step, ahead=ahead,
                          ring_rows=ring_rows, ring_off=ring_off),
        grid=(n_seg // segs_per_step,),
        in_specs=[
            hbm, full((M, D)), hbm, hbm, hbm, hbm, hbm, hbm, full((ks, D)),
            hbm, full((1, D)), full((1, D)), full((2 * T, T)), full((T, 2 * T)),
        ],
        out_specs=pl.BlockSpec((segs_per_step * seg, D), lambda i: (i, 0)),
        out_shape=jax.ShapeDtypeStruct((S, D), A_x.dtype),
        scratch_shapes=[
            pltpu.VMEM((S, D), bf16),
            pltpu.VMEM((S, D), bf16),
            pltpu.VMEM((S, D), bf16),
            pltpu.VMEM((n_chunk, D, T), bf16),
            pltpu.VMEM((N_STAGE, 4, 2 * Dh, D), bf16),
            pltpu.VMEM((3 * E // LANES, D // 2, LANES), u32),
            pltpu.VMEM((E // 2, D), u32),
            pltpu.VMEM((ahead // 2, D), u32),
            ring, ring, ring,
            pltpu.VMEM((S, D), bf16),
            pltpu.VMEM((T // seg, 2 * n_chunk + 1, 2 * seg, D), f32),
            pltpu.VMEM((T // seg, n_chunk, 2 * seg, D), f32),
            pltpu.VMEM((2, T // seg, 2 * seg, D), f32),
            pltpu.VMEM((2 * T, D), f32),
            pltpu.VMEM((M, D), f32),
            pltpu.VMEM((M + seg, E), f32),
            pltpu.SemaphoreType.DMA((2,)),
            pltpu.SemaphoreType.DMA((4, n_chunk)),
            pltpu.SemaphoreType.DMA((3, n_chunk)),
        ],
        compiler_params=pltpu.CompilerParams(
            dimension_semantics=("arbitrary",),
            vmem_limit_bytes=120 * 1024 * 1024,
        ),
    )(
        A_x.reshape(S, D), A_mem0.reshape(M, D),
        head_major(A_Wq), head_major(A_Wk), head_major(A_Wv), A_Wo.reshape(E, D),
        B_k.reshape(S, D), B_v.reshape(S, D), B_shift_k.T, B_ssm_k,
        B_ssm_D.reshape(1, D), gate_w.reshape(1, D),
        jnp.asarray(fwd, dtype=bf16), jnp.asarray(inv, dtype=bf16),
    )
    return out.reshape(B, S, D)
```

```python
import functools

import jax
import jax.numpy as jnp
import numpy as np
from jax import lax
from jax.experimental import pallas as pl
from jax.experimental.pallas import tpu as pltpu

f32 = jnp.float32
u32 = jnp.uint32
bf16 = jnp.bfloat16
NT = (((1,), (1,)), ((), ()))
LANES = 128
T = 128
N_STAGE = 3


def _dft_matrices(blk):
    theta = 2.0 * np.pi * (np.arange(T, dtype=np.float64) + 0.5) / (2 * T)
    ang = theta[:, None] * np.arange(T, dtype=np.float64)[None, :]
    fwd = np.stack([np.cos(ang).reshape(-1, blk, T), -np.sin(ang).reshape(-1, blk, T)], axis=1).reshape(2 * T, T)
    inv = fwd.T / T
    return fwd.astype(np.float32), inv.astype(np.float32)


def _kernel(
    x_hbm, mem0_ref, wq_hbm, wk_hbm, wv_hbm, wo_hbm, bk_hbm, bv_hbm, shift_ref,
    ssmk_hbm, ssmd_ref, gw_ref, fwd_ref, inv_ref,
    o_hbm,
    x_ref, bk_ref, bv_ref, ssmk_ref, stage_ref, w_ref, wo_ref, xh_ref, q_ring, k_ring, v_ring,
    kv_ref, xf_ref, cf_ref, kprev_ref, mem_ref, vec_ref, att_ref, o_ref,
    x_sem, w_sem, c_sem, o_sem,
    *, S, D, H, Dh, M, seg, ahead, ring_rows, ring_off,
):
    L = M + seg
    n_pairs = H // 2
    pw = 2 * Dh
    tpp = pw // LANES
    n_col = D // LANES
    n_chunk = S // T
    fb = 16
    nfb = T // fb
    ybase = 2 * n_chunk - 1
    tok = seg - M
    rings = (q_ring, k_ring, v_ring)
    w_hbm = (wq_hbm, wk_hbm, wv_hbm, wo_hbm)
    n_seg = S // seg

    def lanes(i):
        return slice(i * LANES, (i + 1) * LANES)

    def weight_copies(a):
        wrows = pl.ds(pl.multiple_of(a * pw, pw), pw)
        return [pltpu.make_async_copy(w_hbm[m].at[wrows, :], stage_ref.at[a % N_STAGE, m], w_sem.at[m, a])
                for m in range(4)]

    def conv_copies(a):
        trows = pl.ds(pl.multiple_of(a * T, T), T)
        return [
            pltpu.make_async_copy(bk_hbm.at[trows, :], bk_ref.at[trows, :], c_sem.at[0, a]),
            pltpu.make_async_copy(bv_hbm.at[trows, :], bv_ref.at[trows, :], c_sem.at[1, a]),
            pltpu.make_async_copy(ssmk_hbm.at[:, trows], ssmk_ref.at[a], c_sem.at[2, a]),
        ]

    def prologue():
        x_head = pltpu.make_async_copy(x_hbm.at[0:ahead, :], x_ref.at[0:ahead, :], x_sem.at[0])
        x_tail = pltpu.make_async_copy(x_hbm.at[ahead:S, :], x_ref.at[ahead:S, :], x_sem.at[1])
        x_head.start()
        for cp in weight_copies(0) + conv_copies(0):
            cp.start()

        def zero(a, c):
            for q in range(nfb):
                xf_ref[q, a] = jnp.zeros(xf_ref.shape[2:], f32)
            return c

        lax.fori_loop(0, n_chunk - 1, zero, 0)
        kprev_ref[...] = jnp.zeros(kprev_ref.shape, f32)
        mem_ref[...] = mem0_ref[...].astype(f32)
        vec_ref[0:1, :] = ssmd_ref[...].astype(f32).reshape(1, D)
        vec_ref[1:2, :] = gw_ref[...].astype(f32).reshape(1, D)

        def forward_k(a):
            sgn = jnp.where((lax.broadcasted_iota(jnp.int32, (fb, LANES), 0) & 1) == 0, 1.0, -1.0)
            for cg in range(n_col):
                cs = lanes(cg)
                kf = lax.dot_general(fwd_ref[...], ssmk_ref[a, cs, :], NT, preferred_element_type=f32)
                for q in range(nfb):
                    re, im = slice(2 * q * fb, (2 * q + 1) * fb), slice((2 * q + 1) * fb, (2 * q + 2) * fb)
                    cf_ref[q, a, 0:fb, cs] = kf[re] - sgn * kprev_ref[im, cs]
                    cf_ref[q, a, fb:2 * fb, cs] = kf[im] + sgn * kprev_ref[re, cs]
                kprev_ref[:, cs] = kf

        def forward_x(a):
            r0 = pl.multiple_of(a * T, T)
            rows = pl.ds(r0, T)
            rp = pl.ds(pl.multiple_of(jnp.maximum(r0 - 16, 0), 16), 16)
            for cg in range(n_col):
                cs = lanes(cg)
                shift = shift_ref[:, cs].astype(f32)
                prev = jnp.where(a > 0, bk_ref[rp, cs].astype(f32)[8:16], 0.0)
                ext = jnp.concatenate([prev, bk_ref[rows, cs].astype(f32)], axis=0)
                ksh = ext[8:8 + T] * shift[0:1]
                for j in range(1, shift.shape[0]):
                    ksh = ksh + ext[8 - j:8 - j + T] * shift[j:j + 1]
                kv = (ksh * bv_ref[rows, cs].astype(f32)).astype(bf16)
                kv_ref[rows, cs] = kv
                xf = jnp.dot(fwd_ref[...], kv, preferred_element_type=f32)
                for q in range(nfb):
                    xf_ref[q, a + n_chunk - 1, :, cs] = xf[2 * q * fb:(2 * q + 2) * fb]

        x_head.wait()
        xh_ref[...] = pltpu.bitcast(x_ref[0:ahead, :], u32)
        for cp in weight_copies(0) + conv_copies(0):
            cp.wait()
        for a in range(1, N_STAGE - 1):
            for cp in weight_copies(a) + conv_copies(a):
                cp.start()

        def chunk(a, c):
            @pl.when(a + N_STAGE - 1 < n_chunk)
            def _():
                for cp in weight_copies(a + N_STAGE - 1) + conv_copies(a + N_STAGE - 1):
                    cp.start()

            @pl.when(a == n_chunk - N_STAGE + 1)
            def _():
                x_tail.start()

            @pl.when(a > 0)
            def _():
                for cp in weight_copies(a) + conv_copies(a):
                    cp.wait()

            slot = a % N_STAGE
            wo_ref[pl.ds(pl.multiple_of(a * (pw // 2), pw // 2), pw // 2), :] = pltpu.bitcast(
                stage_ref[slot, 3], u32)
            n_blk = 3 * tpp
            mb = 512
            nrb = ahead // mb
            for blk in range(n_blk):
                m, t = divmod(blk, tpp)
                raw = stage_ref[slot, m, lanes(t), :]
                w_ref[a * n_blk + blk] = pltpu.bitcast(raw.T, u32)
                for rb in range(nrb):
                    xh = pltpu.bitcast(xh_ref[rb * mb // 2:(rb + 1) * mb // 2, :], bf16)
                    y = lax.dot_general(xh, raw, NT, preferred_element_type=f32)
                    rings[m][a * tpp + t, ring_off + rb * mb:ring_off + (rb + 1) * mb, :] = y.astype(bf16)
                if blk == 1:
                    forward_k(a)
                if blk == 4:
                    forward_x(a)
            return c

        lax.fori_loop(0, n_chunk, chunk, 0)

        def first(q, c):
            re, im = slice(0, fb), slice(fb, 2 * fb)
            c0r, c0i, c1r, c1i = cf_ref[q, 0, re], cf_ref[q, 0, im], cf_ref[q, 1, re], cf_ref[q, 1, im]
            x0r, x0i = xf_ref[q, n_chunk - 1, re], xf_ref[q, n_chunk - 1, im]
            x1r, x1i = xf_ref[q, n_chunk, re], xf_ref[q, n_chunk, im]
            xf_ref[q, ybase, re] = c0r * x0r - c0i * x0i
            xf_ref[q, ybase, im] = c0r * x0i + c0i * x0r
            xf_ref[q, ybase + 1, re] = (c0r * x1r - c0i * x1i) + (c1r * x0r - c1i * x0i)
            xf_ref[q, ybase + 1, im] = (c0r * x1i + c0i * x1r) + (c1r * x0i + c1i * x0r)
            return c

        lax.fori_loop(0, nfb, first, 0)
        x_tail.wait()

    prologue()

    def step(s, carry):
        r_glb = pl.multiple_of(s * seg, seg)
        rd = pl.ds(pl.multiple_of(lax.rem(s * seg + ring_off, ring_rows), seg), seg)
        wr = pl.ds(pl.multiple_of(lax.rem(s * tok, ring_rows), 8), tok)
        x_new = x_ref[pl.ds(pl.multiple_of(ahead + s * tok, 8), tok), :]
        lhs = jnp.concatenate([mem_ref[...], x_new.astype(f32)], axis=0).astype(bf16)

        half = LANES // 2
        row = lax.broadcasted_iota(jnp.int32, (L, LANES), 0)
        lane = lax.broadcasted_iota(jnp.int32, (L, LANES), 1)
        key = lane & (half - 1)
        is_key = key < L
        allowed = (row < M) | (key >= seg) | (row - M >= key)
        first = lane < half
        first_k = lax.broadcasted_iota(jnp.int32, (half, LANES), 1) < half
        zhalf = jnp.zeros((half, LANES), bf16)
        row_first = lax.broadcasted_iota(jnp.int32, (LANES, LANES), 0) < half
        col_first = lax.broadcasted_iota(jnp.int32, (LANES, LANES), 1) < half

        def proj(p, m):
            out = []
            for t in range(tpp):
                y = jnp.dot(lhs, pltpu.bitcast(w_ref[(p * 3 + m) * tpp + t], bf16), preferred_element_type=f32)
                rings[m][p * tpp + t, wr, :] = y[M:].astype(bf16)
                out.append(y[0:M])
            return out

        def load(p, m):
            return [rings[m][p * tpp + t, rd, :] for t in range(tpp)]

        def keys(tok3, mem3):
            return [
                jnp.concatenate(
                    [tk, jnp.concatenate([mm, jnp.zeros((half - L, LANES), f32)], axis=0).astype(bf16)],
                    axis=0)
                for tk, mm in zip(tok3, mem3)]

        def blockdiag(tok3, mem3):
            a, mid, b = keys(tok3, mem3)
            zero = jnp.zeros_like(mid)
            return (
                jnp.concatenate([a, zhalf], axis=0),
                jnp.concatenate([jnp.where(first_k, mid, zero), jnp.where(first_k, zero, mid)], axis=0),
                jnp.concatenate([zhalf, b], axis=0),
            )

        def keys_t(k_tok, k_mem):
            a, mid, b = keys(k_tok, k_mem)
            outer = jnp.concatenate([a, b], axis=0).T
            inner = jnp.concatenate([mid, mid], axis=0).T
            return outer, inner

        def scores(q_tok, q_mem, kt):
            outer, inner = kt
            zero = jnp.zeros_like(outer)
            kb = (jnp.where(col_first, outer, zero), jnp.where(col_first == row_first, inner, zero),
                  jnp.where(col_first, zero, outer))
            acc = None
            for t in range(tpp):
                q = jnp.concatenate([q_mem[t], q_tok[t].astype(f32)], axis=0)
                y = jnp.dot(q, kb[t], preferred_element_type=f32)
                acc = y if acc is None else acc + y
            return acc

        def softmax(sc):
            sc = jnp.where(allowed, sc * (Dh ** -0.5), -1000000000.0)
            ninf = -jnp.inf
            m0 = jnp.max(jnp.where(first & is_key, sc, ninf), axis=1, keepdims=True)
            m1 = jnp.max(jnp.where(is_key & ~first, sc, ninf), axis=1, keepdims=True)
            e = jnp.exp(jnp.where(is_key, sc - jnp.where(first, m0, m1), ninf))
            s0 = jnp.sum(jnp.where(first, e, 0.0), axis=1, keepdims=True)
            s1 = jnp.sum(jnp.where(first, 0.0, e), axis=1, keepdims=True)
            return e / jnp.where(first, s0, s1)

        def attend(prob, v_tok, v_mem, p):
            vb = blockdiag(v_tok, v_mem)
            for t in range(tpp):
                att_ref[:, lanes(p * tpp + t)] = jnp.dot(prob, vb[t], preferred_element_type=f32)

        pair_id, part = s // nfb, s % nfb
        nxt = jnp.minimum(2 * pair_id + 2, n_chunk - 2)
        c_now = cf_ref.at[part]
        x_now = xf_ref.at[part, pl.ds(nxt, n_chunk + 1)]
        y_now = xf_ref.at[part, pl.ds(ybase + 2 * ((pair_id + 1) % 2), 2)]

        def mac(ft, cg):
            re, im, cs = slice(ft * 8, ft * 8 + 8), slice(fb + ft * 8, fb + ft * 8 + 8), lanes(cg)
            y = [[None, None], [None, None]]
            hi = x_now[n_chunk, re, cs], x_now[n_chunk, im, cs]
            for dl in range(n_chunk):
                cr, ci = c_now[dl, re, cs], c_now[dl, im, cs]
                lo = x_now[n_chunk - 1 - dl, re, cs], x_now[n_chunk - 1 - dl, im, cs]
                for acc, (xr, xi) in zip(y, (lo, hi)):
                    tr = cr * xr - ci * xi
                    ti = cr * xi + ci * xr
                    acc[0] = tr if acc[0] is None else acc[0] + tr
                    acc[1] = ti if acc[1] is None else acc[1] + ti
                hi = lo
                if (dl + 1) % 2 == 0 and dl + 1 < n_chunk:
                    y_now[1, im, cs] = y[1][1]
            for j in range(2):
                y_now[j, re, cs] = y[j][0]
                y_now[j, im, cs] = y[j][1]

        def branch_b():
            rows = pl.ds(r_glb, seg)
            inv = inv_ref[pl.ds(pl.multiple_of((s * seg) % T, seg), seg), :]
            x = x_ref[rows, :].astype(f32)
            z = jnp.sum(x * vec_ref[1:2, :], axis=1, keepdims=True)
            gate = jnp.broadcast_to(jax.nn.sigmoid(z), (seg, LANES))
            out = []
            for cg in range(n_col):
                cs = lanes(cg)
                y = jnp.dot(inv, xf_ref[:, ybase + ((s * seg) // T) % 4, :, cs].reshape(2 * T, LANES).astype(bf16), preferred_element_type=f32)
                y = y + kv_ref[rows, cs].astype(f32) * vec_ref[0:1, cs]
                out.append((1.0 - gate) * (x[:, cs] * y))
            return gate, out

        todo = [(ft, cg) for cg in range(n_col) for ft in range(fb // 8)]
        mac_lo, mac_hi = 10, 58
        accs = [None] * n_col

        def out_proj(p0, p1):
            for n in range(n_col):
                y = jnp.dot(att_ref[:, p0 * pw:p1 * pw], pltpu.bitcast(wo_ref[p0 * pw // 2:p1 * pw // 2, lanes(n)], bf16),
                            preferred_element_type=f32)
                accs[n] = y if accs[n] is None else accs[n] + y

        d_kt, d_sc, d_sm, d_pv = 3, 7, 9, 13
        woc = 1
        qm, km, vm, kt, sc, pr = {}, {}, {}, {}, {}, {}
        done = 0

        def due(u, d):
            p, r = divmod(u - d, 3)
            return p if r == 0 and 0 <= p < n_pairs else None

        for u in range(3 * n_pairs + d_pv - 2):
            p_kt, p_sc, p_sm, p_pv = due(u, d_kt), due(u, d_sc), due(u, d_sm), due(u, d_pv)
            if p_kt is not None:
                k_tok = load(p_kt, 1)
            if p_sc is not None:
                q_tok = load(p_sc, 0)
            if p_pv is not None:
                v_tok = load(p_pv, 2)
            i, r = divmod(u, 3)
            if i < n_pairs:
                (km, qm, vm)[r][i] = proj(i, (1, 0, 2)[r])
            else:
                out_proj(done, done + woc)
                done += woc
            if p_sc is not None:
                sc[p_sc] = scores(q_tok, qm[p_sc], kt[p_sc])
            if p_pv is not None:
                attend(pr[p_pv], v_tok, vm[p_pv], p_pv)
            if p_kt is not None:
                kt[p_kt] = keys_t(k_tok, km[p_kt])
            if p_sm is not None:
                pr[p_sm] = softmax(sc[p_sm])
            if u == 3:
                gate, bt = branch_b()
            if u == -1:
                y_now[0, 0:8, 0:LANES] = (km, qm, vm)[r][i][0]
            if mac_lo <= u < mac_hi and not 0:
                n = len(todo)
                for ft, cg in todo[(u - mac_lo) * n // (mac_hi - mac_lo):(u + 1 - mac_lo) * n // (mac_hi - mac_lo)]:
                    mac(ft, cg)
        out_proj(done, n_pairs)

        for n in range(n_col):
            cs = lanes(n)
            mem_ref[:, cs] = accs[n][0:M]
            res = gate * accs[n][M:L] + bt[n]
            o_ref[pl.ds(r_glb, seg), cs] = res.astype(o_ref.dtype)
        return carry

    grp = 4

    def steps(j, carry):
        lax.fori_loop(j * grp, (j + 1) * grp, step, 0)
        rows = pl.ds(pl.multiple_of(j * grp * seg, grp * seg), grp * seg)
        pltpu.make_async_copy(o_ref.at[rows, :], o_hbm.at[rows, :], o_sem).start()
        return carry

    lax.fori_loop(0, n_seg // grp, steps, 0)
    pltpu.make_async_copy(o_ref, o_hbm, o_sem).wait()


@functools.partial(jax.jit, static_argnames=("A_seg_len",))
def pallas_gated_mix__memory_aug_recurrent_mem_tr__ssm_conv_h3__prompt_kernel(
    A_x: jax.Array,
    A_mem0: jax.Array,
    A_Wq: jax.Array,
    A_Wk: jax.Array,
    A_Wv: jax.Array,
    A_Wo: jax.Array,
    A_seg_len: int,
    B_q: jax.Array,
    B_k: jax.Array,
    B_v: jax.Array,
    B_shift_k: jax.Array,
    B_ssm_k: jax.Array,
    B_ssm_D: jax.Array,
    gate_w: jax.Array,
):
    del B_q
    B, S, D = A_x.shape
    H, Dh = A_Wq.shape[1], A_Wq.shape[2]
    M = A_mem0.shape[1]
    seg = int(A_seg_len)
    n_seg = S // seg
    E = H * Dh
    n_chunk = S // T
    ahead = n_seg * M
    ring_rows, ring_off = 576, 64
    assert (B, S, M, seg, H // 2, 2 * Dh) == (1, 2048, 8, 32, n_chunk, 3 * LANES) and D % LANES == 0

    def head_major(w):
        return jnp.transpose(w, (1, 2, 0)).reshape(E, D)

    fwd, inv = _dft_matrices(16)
    hbm = pl.BlockSpec(memory_space=pl.ANY)

    vmem = pl.BlockSpec(memory_space=pltpu.VMEM)

    ring = pltpu.VMEM((E // LANES, ring_rows, LANES), bf16)
    out = pl.pallas_call(
        functools.partial(_kernel, S=S, D=D, H=H, Dh=Dh, M=M, seg=seg,
                          ahead=ahead,
                          ring_rows=ring_rows, ring_off=ring_off),
        in_specs=[
            hbm, vmem, hbm, hbm, hbm, hbm, hbm, hbm, vmem, hbm, vmem, vmem, vmem, vmem,
        ],
        out_specs=hbm,
        out_shape=jax.ShapeDtypeStruct((S, D), A_x.dtype),
        scratch_shapes=[
            pltpu.VMEM((S, D), bf16),
            pltpu.VMEM((S, D), bf16),
            pltpu.VMEM((S, D), bf16),
            pltpu.VMEM((n_chunk, D, T), bf16),
            pltpu.VMEM((N_STAGE, 4, 2 * Dh, D), bf16),
            pltpu.VMEM((3 * E // LANES, D // 2, LANES), u32),
            pltpu.VMEM((E // 2, D), u32),
            pltpu.VMEM((ahead // 2, D), u32),
            ring, ring, ring,
            pltpu.VMEM((S, D), bf16),
            pltpu.VMEM((T // 16, 2 * n_chunk + 3, 32, D), f32),
            pltpu.VMEM((T // 16, n_chunk, 32, D), f32),
            pltpu.VMEM((2 * T, D), f32),
            pltpu.VMEM((M, D), f32),
            pltpu.VMEM((2, D), f32),
            pltpu.VMEM((M + seg, E), f32),
            pltpu.VMEM((S, D), A_x.dtype),
            pltpu.SemaphoreType.DMA((2,)),
            pltpu.SemaphoreType.DMA((4, n_chunk)),
            pltpu.SemaphoreType.DMA((3, n_chunk)),
            pltpu.SemaphoreType.DMA(()),
        ],
        compiler_params=pltpu.CompilerParams(
            vmem_limit_bytes=120 * 1024 * 1024,
            disable_bounds_checks=bool(1),
        ),
    )(
        A_x.reshape(S, D), A_mem0.reshape(M, D),
        head_major(A_Wq), head_major(A_Wk), head_major(A_Wv), A_Wo.reshape(E, D),
        B_k.reshape(S, D), B_v.reshape(S, D), B_shift_k.T, B_ssm_k,
        B_ssm_D, gate_w,
        jnp.asarray(fwd, dtype=bf16), jnp.asarray(inv, dtype=bf16),
    )
    return out.reshape(B, S, D)
```

```python
import functools

import jax
import jax.numpy as jnp
import numpy as np
from jax import lax
from jax.experimental import pallas as pl
from jax.experimental.pallas import tpu as pltpu

f32 = jnp.float32
u32 = jnp.uint32
bf16 = jnp.bfloat16
NT = (((1,), (1,)), ((), ()))
LANES = 128
T = 128
N_STAGE = 3
UNROLL = 2
FB = 16 * UNROLL
OUT_STEPS = 2


def _dft_matrices():
    theta = 2.0 * np.pi * (np.arange(T, dtype=np.float64) + 0.5) / (2 * T)
    ang = theta[:, None] * np.arange(T, dtype=np.float64)[None, :]
    fwd = np.stack([np.cos(ang).reshape(-1, FB, T), -np.sin(ang).reshape(-1, FB, T)], axis=1)
    fwd = fwd.reshape(2 * T, T)
    return fwd.astype(np.float32), (fwd.T / T).astype(np.float32)


def _dot(a, b):
    return jnp.dot(a, b, preferred_element_type=f32)


def _lanes(i):
    return slice(i * LANES, (i + 1) * LANES)


def _cmul(ar, ai, br, bi):
    return ar * br - ai * bi, ar * bi + ai * br


def _kernel(
    x_hbm, mem0_ref, wq_hbm, wk_hbm, wv_hbm, wo_hbm, bk_hbm, bv_hbm, shift_ref,
    ssmk_hbm, ssmd_ref, gw_ref, fwd_ref, inv_ref,
    o_hbm,
    x_ref, bk_ref, bv_ref, ssmk_ref, stage_ref, w_ref, wo_ref, xh_ref, q_ring, k_ring, v_ring,
    kv_ref, xf_ref, cf_ref, kprev_ref, vec_ref, att_ref, o_ref,
    x_sem, w_sem, c_sem, o_sem,
    *, S, D, H, Dh, M, seg, ahead, ring_rows, ring_off,
):
    L = M + seg
    n_seg = S // seg
    n_pairs = H // 2
    pw = 2 * Dh
    tpp = pw // LANES
    n_col = D // LANES
    n_chunk = S // T
    nfb = T // FB
    xbase = n_chunk - 1
    ybase = xbase + n_chunk
    tok = seg - M
    rings = (q_ring, k_ring, v_ring)
    w_hbm = (wq_hbm, wk_hbm, wv_hbm, wo_hbm)
    re_blk, im_blk = slice(0, FB), slice(FB, 2 * FB)

    def chunk_copies(a):
        wrows = pl.ds(pl.multiple_of(a * pw, pw), pw)
        trows = pl.ds(pl.multiple_of(a * T, T), T)
        return [
            pltpu.make_async_copy(w_hbm[m].at[wrows, :], stage_ref.at[a % N_STAGE, m], w_sem.at[m, a])
            for m in range(4)
        ] + [
            pltpu.make_async_copy(bk_hbm.at[trows, :], bk_ref.at[trows, :], c_sem.at[0, a]),
            pltpu.make_async_copy(bv_hbm.at[trows, :], bv_ref.at[trows, :], c_sem.at[1, a]),
            pltpu.make_async_copy(ssmk_hbm.at[:, trows], ssmk_ref.at[a], c_sem.at[2, a]),
        ]

    x_head = pltpu.make_async_copy(x_hbm.at[0:ahead, :], x_ref.at[0:ahead, :], x_sem.at[0])
    x_tail = pltpu.make_async_copy(x_hbm.at[ahead:S, :], x_ref.at[ahead:S, :], x_sem.at[1])
    x_head.start()
    for cp in chunk_copies(0):
        cp.start()

    def zero(a, c):
        for q in range(nfb):
            xf_ref[q, a] = jnp.zeros(xf_ref.shape[2:], f32)
        return c

    lax.fori_loop(0, xbase, zero, 0)
    kprev_ref[...] = jnp.zeros(kprev_ref.shape, f32)
    vec_ref[0:1, :] = ssmd_ref[...].astype(f32).reshape(1, D)
    vec_ref[1:2, :] = gw_ref[...].astype(f32).reshape(1, D)
    x_head.wait()
    xh_ref[...] = pltpu.bitcast(x_ref[0:ahead, :], u32)
    for cp in chunk_copies(0):
        cp.wait()
    for a in range(1, N_STAGE):
        for cp in chunk_copies(a):
            cp.start()

    def spectrum_ssm(a):
        sgn = jnp.where((lax.broadcasted_iota(jnp.int32, (FB, LANES), 0) & 1) == 0, 1.0, -1.0)
        for cg in range(n_col):
            cs = _lanes(cg)
            kf = lax.dot_general(fwd_ref[...], ssmk_ref[a, cs, :], NT, preferred_element_type=f32)
            for q in range(nfb):
                re, im = slice(2 * q * FB, (2 * q + 1) * FB), slice((2 * q + 1) * FB, (2 * q + 2) * FB)
                cf_ref[q, a, re_blk, cs] = kf[re] - sgn * kprev_ref[im, cs]
                cf_ref[q, a, im_blk, cs] = kf[im] + sgn * kprev_ref[re, cs]
            kprev_ref[:, cs] = kf

    def spectrum_kv(a):
        r0 = pl.multiple_of(a * T, T)
        rows = pl.ds(r0, T)
        before = pl.ds(pl.multiple_of(jnp.maximum(r0 - 16, 0), 16), 16)
        for cg in range(n_col):
            cs = _lanes(cg)
            shift = shift_ref[:, cs].astype(f32)
            prev = jnp.where(a > 0, bk_ref[before, cs].astype(f32)[8:16], 0.0)
            ext = jnp.concatenate([prev, bk_ref[rows, cs].astype(f32)], axis=0)
            ksh = ext[8:8 + T] * shift[0:1]
            for j in range(1, shift.shape[0]):
                ksh = ksh + ext[8 - j:8 - j + T] * shift[j:j + 1]
            kv = (ksh * bv_ref[rows, cs].astype(f32)).astype(bf16)
            kv_ref[rows, cs] = kv
            xf = _dot(fwd_ref[...], kv)
            for q in range(nfb):
                xf_ref[q, xbase + a, :, cs] = xf[2 * q * FB:(2 * q + 2) * FB]

    def chunk(a, c):
        @pl.when(a > 0)
        def _():
            for cp in chunk_copies(a):
                cp.wait()

        slot = a % N_STAGE
        for blk in range(3 * tpp):
            m, t = divmod(blk, tpp)
            if blk == 3:
                wo_rows = pl.ds(pl.multiple_of(a * (pw // 2), pw // 2), pw // 2)
                wo_ref[wo_rows, :] = pltpu.bitcast(stage_ref[slot, 3], u32)
            raw = stage_ref[slot, m, _lanes(t), :]
            w_ref[a * 3 * tpp + blk] = pltpu.bitcast(raw.T, u32)
            y = lax.dot_general(pltpu.bitcast(xh_ref[...], bf16), raw, NT, preferred_element_type=f32)
            rings[m][a * tpp + t, ring_off:ring_off + ahead, :] = y.astype(bf16)
            if blk == 3:
                spectrum_ssm(a)
            if blk == 5:
                spectrum_kv(a)

        @pl.when(a + N_STAGE < n_chunk)
        def _():
            for cp in chunk_copies(a + N_STAGE):
                cp.start()

        @pl.when(a == n_chunk - N_STAGE)
        def _():
            x_tail.start()

        return c

    lax.fori_loop(0, n_chunk, chunk, 0)

    def first_outputs(q, c):
        c0 = cf_ref[q, 0, re_blk], cf_ref[q, 0, im_blk]
        c1 = cf_ref[q, 1, re_blk], cf_ref[q, 1, im_blk]
        x0 = xf_ref[q, xbase, re_blk], xf_ref[q, xbase, im_blk]
        x1 = xf_ref[q, xbase + 1, re_blk], xf_ref[q, xbase + 1, im_blk]
        xf_ref[q, ybase, re_blk], xf_ref[q, ybase, im_blk] = _cmul(*c0, *x0)
        (ar, ai), (br, bi) = _cmul(*c0, *x1), _cmul(*c1, *x0)
        xf_ref[q, ybase + 1, re_blk], xf_ref[q, ybase + 1, im_blk] = ar + br, ai + bi
        return c

    lax.fori_loop(0, nfb, first_outputs, 0)
    x_tail.wait()

    def convolve_spectra(it):
        pair_id, part = it // nfb, it % nfb
        nxt = jnp.minimum(2 * pair_id + 2, n_chunk - 2)
        c_now = cf_ref.at[part]
        x_now = xf_ref.at[part, pl.ds(nxt, n_chunk + 1)]
        y_now = xf_ref.at[part, pl.ds(ybase + 2 * ((pair_id + 1) % 2), 2)]
        for cg in range(n_col):
            for ft in range(FB // 8):
                re, im, cs = slice(ft * 8, ft * 8 + 8), slice(FB + ft * 8, FB + ft * 8 + 8), _lanes(cg)
                y = [None, None]
                hi = x_now[n_chunk, re, cs], x_now[n_chunk, im, cs]
                for dl in range(n_chunk):
                    cc = c_now[dl, re, cs], c_now[dl, im, cs]
                    lo = x_now[n_chunk - 1 - dl, re, cs], x_now[n_chunk - 1 - dl, im, cs]
                    for j, xx in enumerate((lo, hi)):
                        tr, ti = _cmul(*cc, *xx)
                        y[j] = (tr, ti) if y[j] is None else (y[j][0] + tr, y[j][1] + ti)
                    hi = lo
                    if (dl + 1) % 3 == 0 and dl + 1 < n_chunk:
                        y_now[1, im, cs] = y[1][1]
                for j in range(2):
                    y_now[j, re, cs], y_now[j, im, cs] = y[j]

    def gate_and_b(it):
        n = UNROLL * seg
        r0 = pl.multiple_of(it * n, n)
        rows = pl.ds(r0, n)
        inv = inv_ref[pl.ds(pl.multiple_of(r0 % T, n), n), :]
        x = x_ref[rows, :].astype(f32)
        z = jnp.sum(x * vec_ref[1:2, :], axis=1, keepdims=True)
        gate = jnp.broadcast_to(jax.nn.sigmoid(z), (n, LANES))
        out = []
        for cg in range(n_col):
            cs = _lanes(cg)
            yf = xf_ref[:, ybase + (r0 // T) % 4, :, cs].reshape(2 * T, LANES)
            y = _dot(inv, yf.astype(bf16)) + kv_ref[rows, cs].astype(f32) * vec_ref[0:1, cs]
            out.append((1.0 - gate) * (x[:, cs] * y))
        return gate, out

    def step(it, sub, mem, shared):
        s = it * UNROLL + sub
        rd = pl.ds(pl.multiple_of(lax.rem(s * seg + ring_off, ring_rows), seg), seg)
        wr = pl.ds(pl.multiple_of(lax.rem(s * tok, ring_rows), 8), tok)
        x_new = x_ref[pl.ds(pl.multiple_of(ahead + s * tok, 8), tok), :]
        lhs = [jnp.concatenate([mem[n], x_new[:, _lanes(n)].astype(f32)], axis=0).astype(bf16)
               for n in range(n_col)]
        lhs_all = jnp.concatenate(lhs, axis=1)

        half = LANES // 2
        row = lax.broadcasted_iota(jnp.int32, (L, LANES), 0)
        lane = lax.broadcasted_iota(jnp.int32, (L, LANES), 1)
        key = lane & (half - 1)
        is_key = key < L
        allowed = (row < M) | (key >= seg) | (row - M >= key)
        first = lane < half
        first_k = lax.broadcasted_iota(jnp.int32, (half, LANES), 1) < half
        zhalf = jnp.zeros((half, LANES), bf16)
        row_first = lax.broadcasted_iota(jnp.int32, (LANES, LANES), 0) < half
        col_first = lax.broadcasted_iota(jnp.int32, (LANES, LANES), 1) < half

        def weights(p, m, t, n0, n1):
            return pltpu.bitcast(w_ref[(p * 3 + m) * tpp + t, n0 * half:n1 * half, :], bf16)

        def proj(p, m, early=0):
            if early:
                ys = [_dot(lhs_all[:, :early * LANES], weights(p, m, t, 0, early)) for t in range(tpp)]
                for n in range(early, n_col):
                    ys = [y + _dot(lhs[n], weights(p, m, t, n, n + 1)) for t, y in enumerate(ys)]
            out = []
            for t in range(tpp):
                y = ys[t] if early else _dot(lhs_all, weights(p, m, t, 0, n_col))
                rings[m][p * tpp + t, wr, :] = y[M:].astype(bf16)
                out.append(y[0:M])
            return out

        def load(p, m):
            return [rings[m][p * tpp + t, rd, :] for t in range(tpp)]

        def keys(tok3, mem3):
            pad = jnp.zeros((half - L, LANES), f32)
            return [jnp.concatenate([tk, jnp.concatenate([mm, pad], axis=0).astype(bf16)], axis=0)
                    for tk, mm in zip(tok3, mem3)]

        def keys_t(k_tok, k_mem):
            a, mid, b = keys(k_tok, k_mem)
            return jnp.concatenate([a, b], axis=0).T, jnp.concatenate([mid, mid], axis=0).T

        def scores(q_tok, q_mem, kt):
            outer, inner = kt
            zero = jnp.zeros_like(outer)
            kb = (jnp.where(col_first, outer, zero),
                  jnp.where(col_first == row_first, inner, zero),
                  jnp.where(col_first, zero, outer))
            acc = None
            for t in range(tpp):
                y = _dot(jnp.concatenate([q_mem[t], q_tok[t].astype(f32)], axis=0), kb[t])
                acc = y if acc is None else acc + y
            return acc

        def softmax(sc):
            sc = jnp.where(allowed, sc * (Dh ** -0.5), -1000000000.0)
            ninf = -jnp.inf
            m0 = jnp.max(jnp.where(first & is_key, sc, ninf), axis=1, keepdims=True)
            m1 = jnp.max(jnp.where(is_key & ~first, sc, ninf), axis=1, keepdims=True)
            e = jnp.exp(jnp.where(is_key, sc - jnp.where(first, m0, m1), ninf))
            s0 = jnp.sum(jnp.where(first, e, 0.0), axis=1, keepdims=True)
            s1 = jnp.sum(jnp.where(first, 0.0, e), axis=1, keepdims=True)
            return e / jnp.where(first, s0, s1)

        def attend(prob, v_tok, v_mem, p):
            a, mid, b = keys(v_tok, v_mem)
            zero = jnp.zeros_like(mid)
            vb = (jnp.concatenate([a, zhalf], axis=0),
                  jnp.concatenate([jnp.where(first_k, mid, zero), jnp.where(first_k, zero, mid)], axis=0),
                  jnp.concatenate([zhalf, b], axis=0))
            for t in range(tpp):
                att_ref[:, _lanes(p * tpp + t)] = _dot(prob, vb[t])

        accs = [None] * n_col

        def out_proj(p0, p1):
            for n in range(n_col):
                y = _dot(att_ref[:, p0 * pw:p1 * pw],
                         pltpu.bitcast(wo_ref[p0 * pw // 2:p1 * pw // 2, _lanes(n)], bf16))
                accs[n] = y if accs[n] is None else accs[n] + y

        d_kt, d_sc, d_sm, d_pv = 3, 7, 8, 13
        mem_qkv, kt, sc, pr = ({}, {}, {}), {}, {}, {}
        done = 0

        def due(u, d):
            p, r = divmod(u - d, 3)
            return p if r == 0 and 0 <= p < n_pairs else None

        for u in range(3 * n_pairs + d_pv - 2):
            p_kt, p_sc, p_sm, p_pv = due(u, d_kt), due(u, d_sc), due(u, d_sm), due(u, d_pv)
            if p_kt is not None:
                k_tok = load(p_kt, 1)
            if p_sc is not None:
                q_tok = load(p_sc, 0)
            if p_pv is not None:
                v_tok = load(p_pv, 2)
            p, r = divmod(u, 3)
            if p < n_pairs:
                m = (1, 0, 2)[r]
                mem_qkv[m][p] = proj(p, m, early=2 if u == 0 and sub > 0 else 0)
            elif done <= (u - d_pv - 1) // 3:
                out_proj(done, done + 1)
                done += 1
            if p_sc is not None:
                sc[p_sc] = scores(q_tok, mem_qkv[0][p_sc], kt[p_sc])
            if p_pv is not None:
                attend(pr[p_pv], v_tok, mem_qkv[2][p_pv], p_pv)
            if p_kt is not None:
                kt[p_kt] = keys_t(k_tok, mem_qkv[1][p_kt])
            if p_sm is not None:
                pr[p_sm] = softmax(sc[p_sm])
            if sub == 0 and u == 2:
                shared.extend(gate_and_b(it))
            if sub == 0 and u == 3:
                convolve_spectra(it)
        out_proj(done, n_pairs)

        gate, gated_b = shared
        mine = slice(sub * seg, (sub + 1) * seg)
        rows = pl.ds(pl.multiple_of(s * seg, seg), seg)
        for n in range(n_col):
            res = gate[mine] * accs[n][M:L] + gated_b[n][mine]
            o_ref[rows, _lanes(n)] = res.astype(o_ref.dtype)
        return [acc[0:M] for acc in accs]

    def steps(it, mem):
        shared = []
        for sub in range(UNROLL):
            mem = step(it, sub, mem, shared)
        return mem

    def steps_and_copy(j, mem):
        per = OUT_STEPS // UNROLL
        mem = steps(j, mem) if per == 1 else lax.fori_loop(j * per, (j + 1) * per, steps, mem)
        rows = pl.ds(pl.multiple_of(j * OUT_STEPS * seg, OUT_STEPS * seg), OUT_STEPS * seg)
        pltpu.make_async_copy(o_ref.at[rows, :], o_hbm.at[rows, :], o_sem).start()
        return mem

    mem0 = [mem0_ref[:, _lanes(n)].astype(f32) for n in range(n_col)]
    lax.fori_loop(0, n_seg // OUT_STEPS, steps_and_copy, mem0)
    pltpu.make_async_copy(o_ref, o_hbm, o_sem).wait()


@functools.partial(jax.jit, static_argnames=("A_seg_len",))
def pallas_gated_mix__memory_aug_recurrent_mem_tr__ssm_conv_h3__prompt_kernel(
    A_x: jax.Array,
    A_mem0: jax.Array,
    A_Wq: jax.Array,
    A_Wk: jax.Array,
    A_Wv: jax.Array,
    A_Wo: jax.Array,
    A_seg_len: int,
    B_q: jax.Array,
    B_k: jax.Array,
    B_v: jax.Array,
    B_shift_k: jax.Array,
    B_ssm_k: jax.Array,
    B_ssm_D: jax.Array,
    gate_w: jax.Array,
):
    del B_q
    B, S, D = A_x.shape
    H, Dh = A_Wq.shape[1], A_Wq.shape[2]
    M = A_mem0.shape[1]
    seg = int(A_seg_len)
    E = H * Dh
    n_chunk = S // T
    assert (B, S, M, seg) == (1, 2048, 8, 32) and (H // 2, 2 * Dh) == (n_chunk, 3 * LANES)
    assert D % LANES == 0 and B_shift_k.shape[1] <= 9
    ahead = (S // seg) * M
    ring_rows, ring_off = 576, 64

    def head_major(w):
        return jnp.transpose(w, (1, 2, 0)).reshape(E, D)

    fwd, inv = _dft_matrices()
    hbm = pl.BlockSpec(memory_space=pl.ANY)
    vmem = pl.BlockSpec(memory_space=pltpu.VMEM)
    ring = pltpu.VMEM((E // LANES, ring_rows, LANES), bf16)
    out = pl.pallas_call(
        functools.partial(_kernel, S=S, D=D, H=H, Dh=Dh, M=M, seg=seg, ahead=ahead,
                          ring_rows=ring_rows, ring_off=ring_off),
        in_specs=[hbm, vmem, hbm, hbm, hbm, hbm, hbm, hbm, vmem, hbm, vmem, vmem, vmem, vmem],
        out_specs=hbm,
        out_shape=jax.ShapeDtypeStruct((S, D), A_x.dtype),
        scratch_shapes=[
            pltpu.VMEM((S, D), bf16),
            pltpu.VMEM((S, D), bf16),
            pltpu.VMEM((S, D), bf16),
            pltpu.VMEM((n_chunk, D, T), bf16),
            pltpu.VMEM((N_STAGE, 4, 2 * Dh, D), bf16),
            pltpu.VMEM((3 * E // LANES, D // 2, LANES), u32),
            pltpu.VMEM((E // 2, D), u32),
            pltpu.VMEM((ahead // 2, D), u32),
            ring, ring, ring,
            pltpu.VMEM((S, D), bf16),
            pltpu.VMEM((T // FB, 2 * n_chunk + 3, 2 * FB, D), f32),
            pltpu.VMEM((T // FB, n_chunk, 2 * FB, D), f32),
            pltpu.VMEM((2 * T, D), f32),
            pltpu.VMEM((2, D), f32),
            pltpu.VMEM((M + seg, E), f32),
            pltpu.VMEM((S, D), A_x.dtype),
            pltpu.SemaphoreType.DMA((2,)),
            pltpu.SemaphoreType.DMA((4, n_chunk)),
            pltpu.SemaphoreType.DMA((3, n_chunk)),
            pltpu.SemaphoreType.DMA(()),
        ],
        compiler_params=pltpu.CompilerParams(
            vmem_limit_bytes=120 * 1024 * 1024,
            disable_bounds_checks=True,
        ),
    )(
        A_x.reshape(S, D), A_mem0.reshape(M, D),
        head_major(A_Wq), head_major(A_Wk), head_major(A_Wv), A_Wo.reshape(E, D),
        B_k.reshape(S, D), B_v.reshape(S, D), B_shift_k.T, B_ssm_k, B_ssm_D, gate_w,
        jnp.asarray(fwd, dtype=bf16), jnp.asarray(inv, dtype=bf16),
    )
    return out.reshape(B, S, D)
```

```python
import functools

import jax
import jax.numpy as jnp
import numpy as np
from jax import lax
from jax.experimental import pallas as pl
from jax.experimental.pallas import tpu as pltpu

f32 = jnp.float32
u32 = jnp.uint32
bf16 = jnp.bfloat16
NT = (((1,), (1,)), ((), ()))
LANES = 128
T = 128
N_STAGE = 3
UNROLL = 2
FB = 16 * UNROLL
OUT_STEPS = 2


def _dft_matrices():
    theta = 2.0 * np.pi * (np.arange(T, dtype=np.float64) + 0.5) / (2 * T)
    ang = theta[:, None] * np.arange(T, dtype=np.float64)[None, :]
    fwd = np.stack([np.cos(ang).reshape(-1, FB, T), -np.sin(ang).reshape(-1, FB, T)], axis=1)
    fwd = fwd.reshape(2 * T, T)
    return fwd.astype(bf16), (fwd.T / T).astype(bf16)


def _dot(a, b):
    return jnp.dot(a, b, preferred_element_type=f32)


def _lanes(i):
    return slice(i * LANES, (i + 1) * LANES)


def _cmul(ar, ai, br, bi):
    return ar * br - ai * bi, ar * bi + ai * br


def _kernel(
    x_hbm, mem0_ref, wq_hbm, wk_hbm, wv_hbm, wo_hbm, bk_hbm, bv_hbm, shift_ref,
    ssmk_hbm, ssmd_ref, gw_ref, fwd_ref, inv_ref,
    o_hbm,
    x_ref, bk_ref, bv_ref, ssmk_ref, stage_ref, w_ref, wo_ref, xh_ref, q_ring, k_ring, v_ring,
    kv_ref, xf_ref, cf_ref, kprev_ref, att_ref, o_ref, vec_ref,
    x_sem, w_sem, c_sem, o_sem,
    *, S, D, H, Dh, M, seg, ahead, ring_rows, ring_off,
):
    L = M + seg
    n_seg = S // seg
    n_pairs = H // 2
    pw = 2 * Dh
    tpp = pw // LANES
    n_col = D // LANES
    n_chunk = S // T
    nfb = T // FB
    xbase = n_chunk - 1
    ybase = xbase + n_chunk
    tok = seg - M
    rings = (q_ring, k_ring, v_ring)
    w_hbm = (wq_hbm, wk_hbm, wv_hbm, wo_hbm)
    re_blk, im_blk = slice(0, FB), slice(FB, 2 * FB)

    def chunk_copies(a):
        wrows = pl.ds(pl.multiple_of(a * pw, pw), pw)
        trows = pl.ds(pl.multiple_of(a * T, T), T)
        return [
            pltpu.make_async_copy(w_hbm[m].at[wrows, :], stage_ref.at[a % N_STAGE, m], w_sem.at[m, a])
            for m in range(4)
        ] + [
            pltpu.make_async_copy(bk_hbm.at[trows, :], bk_ref.at[trows, :], c_sem.at[0, a]),
            pltpu.make_async_copy(bv_hbm.at[trows, :], bv_ref.at[trows, :], c_sem.at[1, a]),
            pltpu.make_async_copy(ssmk_hbm.at[:, trows], ssmk_ref.at[a], c_sem.at[2, a]),
        ]

    x_head = pltpu.make_async_copy(x_hbm.at[0:ahead, :], x_ref.at[0:ahead, :], x_sem.at[0])
    x_tail = pltpu.make_async_copy(x_hbm.at[ahead:S, :], x_ref.at[ahead:S, :], x_sem.at[1])
    x_head.start()
    for cp in chunk_copies(0):
        cp.start()

    def zero(a, c):
        for q in range(nfb):
            xf_ref[q, a] = jnp.zeros(xf_ref.shape[2:], f32)
        return c

    lax.fori_loop(0, xbase, zero, 0)
    kprev_ref[...] = jnp.zeros(kprev_ref.shape, f32)
    vec_ref[0:1, :] = ssmd_ref[...].astype(f32).reshape(1, D)
    vec_ref[1:2, :] = gw_ref[...].astype(f32).reshape(1, D)
    x_head.wait()
    xh_ref[...] = pltpu.bitcast(x_ref[0:ahead, :], u32)
    for cp in chunk_copies(0):
        cp.wait()
    for a in range(1, N_STAGE):
        for cp in chunk_copies(a):
            cp.start()

    def spectrum_ssm(a):
        sgn = jnp.where((lax.broadcasted_iota(jnp.int32, (FB, LANES), 0) & 1) == 0, 1.0, -1.0)
        for cg in range(n_col):
            cs = _lanes(cg)
            kf = lax.dot_general(fwd_ref[...], ssmk_ref[a, cs, :], NT, preferred_element_type=f32)
            for q in range(nfb):
                re, im = slice(2 * q * FB, (2 * q + 1) * FB), slice((2 * q + 1) * FB, (2 * q + 2) * FB)
                cf_ref[q, a, re_blk, cs] = kf[re] - sgn * kprev_ref[im, cs]
                cf_ref[q, a, im_blk, cs] = kf[im] + sgn * kprev_ref[re, cs]
            kprev_ref[:, cs] = kf

    def spectrum_kv(a):
        r0 = pl.multiple_of(a * T, T)
        rows = pl.ds(r0, T)
        before = pl.ds(pl.multiple_of(jnp.maximum(r0 - 16, 0), 16), 16)
        for cg in range(n_col):
            cs = _lanes(cg)
            shift = shift_ref[:, cs].astype(f32)
            prev = jnp.where(a > 0, bk_ref[before, cs].astype(f32)[8:16], 0.0)
            ext = jnp.concatenate([prev, bk_ref[rows, cs].astype(f32)], axis=0)
            ksh = ext[8:8 + T] * shift[0:1]
            for j in range(1, shift.shape[0]):
                ksh = ksh + ext[8 - j:8 - j + T] * shift[j:j + 1]
            kv = (ksh * bv_ref[rows, cs].astype(f32)).astype(bf16)
            kv_ref[rows, cs] = kv
            xf = _dot(fwd_ref[...], kv)
            for q in range(nfb):
                xf_ref[q, xbase + a, :, cs] = xf[2 * q * FB:(2 * q + 2) * FB]

    def chunk(a, c):
        @pl.when(a > 0)
        def _():
            for cp in chunk_copies(a):
                cp.wait()

        slot = a % N_STAGE
        for blk in range(3 * tpp):
            m, t = divmod(blk, tpp)
            if blk == 0:
                wo_rows = pl.ds(pl.multiple_of(a * (pw // 2), pw // 2), pw // 2)
                wo_ref[wo_rows, :] = pltpu.bitcast(stage_ref[slot, 3], u32)
            raw = stage_ref[slot, m, _lanes(t), :]
            w_ref[a * 3 * tpp + blk] = pltpu.bitcast(raw.T, u32)
            y = lax.dot_general(pltpu.bitcast(xh_ref[...], bf16), raw, NT, preferred_element_type=f32)
            rings[m][a * tpp + t, ring_off:ring_off + ahead, :] = y.astype(bf16)
            if blk == 1:
                spectrum_ssm(a)
            if blk == 5:
                spectrum_kv(a)

        @pl.when(a + N_STAGE < n_chunk)
        def _():
            for cp in chunk_copies(a + N_STAGE):
                cp.start()

        @pl.when(a == n_chunk - N_STAGE)
        def _():
            x_tail.start()

        return c

    lax.fori_loop(0, n_chunk, chunk, 0)

    def first_outputs(q, c):
        c0 = cf_ref[q, 0, re_blk], cf_ref[q, 0, im_blk]
        c1 = cf_ref[q, 1, re_blk], cf_ref[q, 1, im_blk]
        x0 = xf_ref[q, xbase, re_blk], xf_ref[q, xbase, im_blk]
        x1 = xf_ref[q, xbase + 1, re_blk], xf_ref[q, xbase + 1, im_blk]
        xf_ref[q, ybase, re_blk], xf_ref[q, ybase, im_blk] = _cmul(*c0, *x0)
        (ar, ai), (br, bi) = _cmul(*c0, *x1), _cmul(*c1, *x0)
        xf_ref[q, ybase + 1, re_blk], xf_ref[q, ybase + 1, im_blk] = ar + br, ai + bi
        return c

    lax.fori_loop(0, nfb, first_outputs, 0)
    x_tail.wait()

    def convolve_spectra(it):
        pair_id, part = it // nfb, it % nfb
        nxt = jnp.minimum(2 * pair_id + 2, n_chunk - 2)
        c_now = cf_ref.at[part]
        x_now = xf_ref.at[part, pl.ds(nxt, n_chunk + 1)]
        y_now = xf_ref.at[part, pl.ds(ybase + 2 * ((pair_id + 1) % 2), 2)]
        for cg in range(n_col):
            for ft in range(FB // 8):
                re, im, cs = slice(ft * 8, ft * 8 + 8), slice(FB + ft * 8, FB + ft * 8 + 8), _lanes(cg)
                y = [None, None]
                hi = x_now[n_chunk, re, cs], x_now[n_chunk, im, cs]
                for dl in range(n_chunk):
                    cc = c_now[dl, re, cs], c_now[dl, im, cs]
                    lo = x_now[n_chunk - 1 - dl, re, cs], x_now[n_chunk - 1 - dl, im, cs]
                    for j, xx in enumerate((lo, hi)):
                        tr, ti = _cmul(*cc, *xx)
                        y[j] = (tr, ti) if y[j] is None else (y[j][0] + tr, y[j][1] + ti)
                    hi = lo
                    if (dl + 1) % 3 == 0 and dl + 1 < n_chunk:
                        y_now[1, im, cs] = y[1][1]
                for j in range(2):
                    y_now[j, re, cs], y_now[j, im, cs] = y[j]

    def gate_and_b(it):
        n = UNROLL * seg
        r0 = pl.multiple_of(it * n, n)
        rows = pl.ds(r0, n)
        inv = inv_ref[pl.ds(pl.multiple_of(r0 % T, n), n), :]
        x = x_ref[rows, :].astype(f32)
        z = jnp.sum(x * vec_ref[1:2, :], axis=1, keepdims=True)
        gate = jnp.broadcast_to(jax.nn.sigmoid(z), (n, LANES))
        out = []
        for cg in range(n_col):
            cs = _lanes(cg)
            yf = xf_ref[:, ybase + (r0 // T) % 4, :, cs].reshape(2 * T, LANES)
            y = _dot(inv, yf.astype(bf16)) + kv_ref[rows, cs].astype(f32) * vec_ref[0:1, cs]
            out.append((1.0 - gate) * (x[:, cs] * y))
        return gate, out

    def step(it, sub, mem, shared):
        s = it * UNROLL + sub
        rd = pl.ds(pl.multiple_of(lax.rem(s * seg + ring_off, ring_rows), seg), seg)
        wr = pl.ds(pl.multiple_of(lax.rem(s * tok, ring_rows), 8), tok)
        x_new = x_ref[pl.ds(pl.multiple_of(ahead + s * tok, 8), tok), :]
        lhs = [jnp.concatenate([mem[n], x_new[:, _lanes(n)].astype(f32)], axis=0).astype(bf16)
               for n in range(n_col)]
        lhs_all = jnp.concatenate(lhs, axis=1)

        half = LANES // 2
        row = lax.broadcasted_iota(jnp.int32, (L, LANES), 0)
        lane = lax.broadcasted_iota(jnp.int32, (L, LANES), 1)
        key = lane & (half - 1)
        is_key = key < L
        allowed = (row < M) | (key >= seg) | (row - M >= key)
        first = lane < half
        first_k = lax.broadcasted_iota(jnp.int32, (half, LANES), 1) < half
        zhalf = jnp.zeros((half, LANES), bf16)
        row_first = lax.broadcasted_iota(jnp.int32, (LANES, LANES), 0) < half
        col_first = lax.broadcasted_iota(jnp.int32, (LANES, LANES), 1) < half

        def weights(p, m, t, n0, n1):
            return pltpu.bitcast(w_ref[(p * 3 + m) * tpp + t, n0 * half:n1 * half, :], bf16)

        def proj(p, m, early=0):
            if early:
                ys = [_dot(lhs_all[:, :early * LANES], weights(p, m, t, 0, early)) for t in range(tpp)]
                for n in range(early, n_col):
                    ys = [y + _dot(lhs[n], weights(p, m, t, n, n + 1)) for t, y in enumerate(ys)]
            out = []
            for t in range(tpp):
                y = ys[t] if early else _dot(lhs_all, weights(p, m, t, 0, n_col))
                rings[m][p * tpp + t, wr, :] = y[M:].astype(bf16)
                out.append(y[0:M])
            return out

        def load(p, m):
            return [rings[m][p * tpp + t, rd, :] for t in range(tpp)]

        def keys(tok3, mem3):
            pad = jnp.zeros((half - L, LANES), f32)
            return [jnp.concatenate([tk, jnp.concatenate([mm, pad], axis=0).astype(bf16)], axis=0)
                    for tk, mm in zip(tok3, mem3)]

        def keys_t(k_tok, k_mem):
            a, mid, b = keys(k_tok, k_mem)
            return jnp.concatenate([a, b], axis=0).T, jnp.concatenate([mid, mid], axis=0).T

        def scores(q_tok, q_mem, kt):
            outer, inner = kt
            zero = jnp.zeros_like(outer)
            kb = (jnp.where(col_first, outer, zero),
                  jnp.where(col_first == row_first, inner, zero),
                  jnp.where(col_first, zero, outer))
            acc = None
            for t in range(tpp):
                y = _dot(jnp.concatenate([q_mem[t], q_tok[t].astype(f32)], axis=0), kb[t])
                acc = y if acc is None else acc + y
            return acc

        def softmax(sc):
            sc = jnp.where(allowed, sc * (Dh ** -0.5), -1000000000.0)
            ninf = -jnp.inf
            m0 = jnp.max(jnp.where(first & is_key, sc, ninf), axis=1, keepdims=True)
            m1 = jnp.max(jnp.where(is_key & ~first, sc, ninf), axis=1, keepdims=True)
            e = jnp.exp(jnp.where(is_key, sc - jnp.where(first, m0, m1), ninf))
            s0 = jnp.sum(jnp.where(first, e, 0.0), axis=1, keepdims=True)
            s1 = jnp.sum(jnp.where(first, 0.0, e), axis=1, keepdims=True)
            return e / jnp.where(first, s0, s1)

        def attend(prob, v_tok, v_mem, p):
            a, mid, b = keys(v_tok, v_mem)
            zero = jnp.zeros_like(mid)
            vb = (jnp.concatenate([a, zhalf], axis=0),
                  jnp.concatenate([jnp.where(first_k, mid, zero), jnp.where(first_k, zero, mid)], axis=0),
                  jnp.concatenate([zhalf, b], axis=0))
            for t in range(tpp):
                att_ref[:, _lanes(p * tpp + t)] = _dot(prob, vb[t])

        accs = [None] * n_col

        def out_proj(p0, p1):
            for n in range(n_col):
                y = _dot(att_ref[:, p0 * pw:p1 * pw],
                         pltpu.bitcast(wo_ref[p0 * pw // 2:p1 * pw // 2, _lanes(n)], bf16))
                accs[n] = y if accs[n] is None else accs[n] + y

        d_kt, d_sc, d_sm, d_pv = 3, 7, 8, 13
        mem_qkv, kt, sc, pr = ({}, {}, {}), {}, {}, {}
        done = 0

        def due(u, d):
            p, r = divmod(u - d, 3)
            return p if r == 0 and 0 <= p < n_pairs else None

        for u in range(3 * n_pairs + d_pv - 2):
            p_kt, p_sc, p_sm, p_pv = due(u, d_kt), due(u, d_sc), due(u, d_sm), due(u, d_pv)
            if p_kt is not None:
                k_tok = load(p_kt, 1)
            if p_sc is not None:
                q_tok = load(p_sc, 0)
            if p_pv is not None:
                v_tok = load(p_pv, 2)
            p, r = divmod(u, 3)
            if p < n_pairs:
                m = (1, 0, 2)[r]
                mem_qkv[m][p] = proj(p, m, early=2 if u == 0 and sub > 0 else 0)
            elif done <= (u - d_pv - 1) // 3:
                out_proj(done, done + 1)
                done += 1
            if p_sc is not None:
                sc[p_sc] = scores(q_tok, mem_qkv[0][p_sc], kt[p_sc])
            if p_pv is not None:
                attend(pr[p_pv], v_tok, mem_qkv[2][p_pv], p_pv)
            if p_kt is not None:
                kt[p_kt] = keys_t(k_tok, mem_qkv[1][p_kt])
            if p_sm is not None:
                pr[p_sm] = softmax(sc[p_sm])
            if sub == 0 and u == 2:
                shared.extend(gate_and_b(it))
            if sub == 0 and u == 3:
                convolve_spectra(it)
        out_proj(done, n_pairs)

        gate, gated_b = shared
        mine = slice(sub * seg, (sub + 1) * seg)
        rows = pl.ds(pl.multiple_of(s * seg, seg), seg)
        for n in range(n_col):
            res = gate[mine] * accs[n][M:L] + gated_b[n][mine]
            o_ref[rows, _lanes(n)] = res.astype(o_ref.dtype)
        return [acc[0:M] for acc in accs]

    def steps(it, mem):
        shared = []
        for sub in range(UNROLL):
            mem = step(it, sub, mem, shared)
        return mem

    def steps_and_copy(j, mem):
        per = OUT_STEPS // UNROLL
        mem = steps(j, mem) if per == 1 else lax.fori_loop(j * per, (j + 1) * per, steps, mem)
        rows = pl.ds(pl.multiple_of(j * OUT_STEPS * seg, OUT_STEPS * seg), OUT_STEPS * seg)
        pltpu.make_async_copy(o_ref.at[rows, :], o_hbm.at[rows, :], o_sem).start()
        return mem

    mem0 = [mem0_ref[:, _lanes(n)].astype(f32) for n in range(n_col)]
    lax.fori_loop(0, n_seg // OUT_STEPS, steps_and_copy, mem0)
    pltpu.make_async_copy(o_ref, o_hbm, o_sem).wait()


@functools.partial(jax.jit, static_argnames=("A_seg_len",))
def pallas_gated_mix__memory_aug_recurrent_mem_tr__ssm_conv_h3__prompt_kernel(
    A_x: jax.Array,
    A_mem0: jax.Array,
    A_Wq: jax.Array,
    A_Wk: jax.Array,
    A_Wv: jax.Array,
    A_Wo: jax.Array,
    A_seg_len: int,
    B_q: jax.Array,
    B_k: jax.Array,
    B_v: jax.Array,
    B_shift_k: jax.Array,
    B_ssm_k: jax.Array,
    B_ssm_D: jax.Array,
    gate_w: jax.Array,
):
    del B_q
    B, S, D = A_x.shape
    H, Dh = A_Wq.shape[1], A_Wq.shape[2]
    M = A_mem0.shape[1]
    seg = int(A_seg_len)
    E = H * Dh
    n_chunk = S // T
    assert (B, S, M, seg) == (1, 2048, 8, 32) and (H // 2, 2 * Dh) == (n_chunk, 3 * LANES)
    assert D % LANES == 0 and B_shift_k.shape[1] <= 9
    ahead = (S // seg) * M
    ring_rows, ring_off = 576, 64

    def head_major(w):
        return jnp.transpose(w, (1, 2, 0)).reshape(E, D)

    fwd, inv = _dft_matrices()
    hbm = pl.BlockSpec(memory_space=pl.ANY)
    vmem = pl.BlockSpec(memory_space=pltpu.VMEM)
    ring = pltpu.VMEM((E // LANES, ring_rows, LANES), bf16)
    out = pl.pallas_call(
        functools.partial(_kernel, S=S, D=D, H=H, Dh=Dh, M=M, seg=seg, ahead=ahead,
                          ring_rows=ring_rows, ring_off=ring_off),
        in_specs=[hbm, vmem, hbm, hbm, hbm, hbm, hbm, hbm, vmem, hbm, vmem, vmem, vmem, vmem],
        out_specs=hbm,
        out_shape=jax.ShapeDtypeStruct((S, D), A_x.dtype),
        scratch_shapes=[
            pltpu.VMEM((S, D), bf16),
            pltpu.VMEM((S, D), bf16),
            pltpu.VMEM((S, D), bf16),
            pltpu.VMEM((n_chunk, D, T), bf16),
            pltpu.VMEM((N_STAGE, 4, 2 * Dh, D), bf16),
            pltpu.VMEM((3 * E // LANES, D // 2, LANES), u32),
            pltpu.VMEM((E // 2, D), u32),
            pltpu.VMEM((ahead // 2, D), u32),
            ring, ring, ring,
            pltpu.VMEM((S, D), bf16),
            pltpu.VMEM((T // FB, 2 * n_chunk + 3, 2 * FB, D), f32),
            pltpu.VMEM((T // FB, n_chunk, 2 * FB, D), f32),
            pltpu.VMEM((2 * T, D), f32),
            pltpu.VMEM((M + seg, E), f32),
            pltpu.VMEM((S, D), A_x.dtype),
            pltpu.VMEM((2, D), f32),
            pltpu.SemaphoreType.DMA((2,)),
            pltpu.SemaphoreType.DMA((4, n_chunk)),
            pltpu.SemaphoreType.DMA((3, n_chunk)),
            pltpu.SemaphoreType.DMA(()),
        ],
        compiler_params=pltpu.CompilerParams(
            vmem_limit_bytes=120 * 1024 * 1024,
            disable_bounds_checks=True,
        ),
    )(
        A_x.reshape(S, D), A_mem0.reshape(M, D),
        head_major(A_Wq), head_major(A_Wk), head_major(A_Wv), A_Wo.reshape(E, D),
        B_k.reshape(S, D), B_v.reshape(S, D), B_shift_k.T, B_ssm_k, B_ssm_D, gate_w,
        fwd, inv,
    )
    return out.reshape(B, S, D)
```

```python
import functools
import math

import jax
import jax.numpy as jnp
import numpy as np
from jax import lax
from jax.experimental import pallas as pl
from jax.experimental.pallas import tpu as pltpu

f32 = jnp.float32
u32 = jnp.uint32
bf16 = jnp.bfloat16
NT = (((1,), (1,)), ((), ()))
LANES = 128
T = 128
N_STAGE = 3
UNROLL = 2
FB = 16 * UNROLL
OUT_STEPS = 2


def _dft_matrices():
    theta = 2.0 * np.pi * (np.arange(T, dtype=np.float64) + 0.5) / (2 * T)
    ang = theta[:, None] * np.arange(T, dtype=np.float64)[None, :]
    fwd = np.stack([np.cos(ang).reshape(-1, FB, T), -np.sin(ang).reshape(-1, FB, T)], axis=1)
    fwd = fwd.reshape(2 * T, T)
    return fwd.astype(bf16), (fwd.T / T).astype(bf16)


def _dot(a, b):
    return jnp.dot(a, b, preferred_element_type=f32)


def _lanes(i):
    return slice(i * LANES, (i + 1) * LANES)


def _cmul(ar, ai, br, bi):
    return ar * br - ai * bi, ar * bi + ai * br


def _kernel(
    x_hbm, mem0_ref, wq_hbm, wk_hbm, wv_hbm, wo_hbm, bk_hbm, bv_hbm, shift_ref,
    ssmk_hbm, ssmd_ref, gw_ref, fwd_ref, inv_ref,
    o_hbm,
    x_ref, bk_ref, bv_ref, ssmk_ref, stage_ref, w_ref, wo_ref, xh_ref, q_ring, k_ring, v_ring,
    kv_ref, xf_ref, cf_ref, kprev_ref, att_ref, o_ref, vec_ref,
    x_sem, w_sem, c_sem, o_sem,
    *, S, D, H, Dh, M, seg, ahead, ring_rows, ring_off,
):
    L = M + seg
    n_seg = S // seg
    n_pairs = H // 2
    pw = 2 * Dh
    tpp = pw // LANES
    n_col = D // LANES
    n_chunk = S // T
    nfb = T // FB
    xbase = n_chunk - 1
    ybase = xbase + n_chunk
    tok = seg - M
    rings = (q_ring, k_ring, v_ring)
    w_hbm = (wq_hbm, wk_hbm, wv_hbm, wo_hbm)
    re_blk, im_blk = slice(0, FB), slice(FB, 2 * FB)

    def chunk_copies(a):
        wrows = pl.ds(pl.multiple_of(a * pw, pw), pw)
        trows = pl.ds(pl.multiple_of(a * T, T), T)
        return [
            pltpu.make_async_copy(w_hbm[m].at[wrows, :], stage_ref.at[a % N_STAGE, m], w_sem.at[m, a])
            for m in range(4)
        ] + [
            pltpu.make_async_copy(bk_hbm.at[trows, :], bk_ref.at[trows, :], c_sem.at[0, a]),
            pltpu.make_async_copy(bv_hbm.at[trows, :], bv_ref.at[trows, :], c_sem.at[1, a]),
            pltpu.make_async_copy(ssmk_hbm.at[:, trows], ssmk_ref.at[a], c_sem.at[2, a]),
        ]

    x_head = pltpu.make_async_copy(x_hbm.at[0:ahead, :], x_ref.at[0:ahead, :], x_sem.at[0])
    x_tail = pltpu.make_async_copy(x_hbm.at[ahead:S, :], x_ref.at[ahead:S, :], x_sem.at[1])
    x_head.start()
    for cp in chunk_copies(0):
        cp.start()

    def zero(a, c):
        for q in range(nfb):
            xf_ref[q, a] = jnp.zeros(xf_ref.shape[2:], f32)
        return c

    lax.fori_loop(0, xbase, zero, 0)
    kprev_ref[...] = jnp.zeros(kprev_ref.shape, f32)
    vec_ref[0:1, :] = ssmd_ref[...].astype(f32).reshape(1, D)
    vec_ref[1:2, :] = gw_ref[...].astype(f32).reshape(1, D)
    x_head.wait()
    xh_ref[...] = pltpu.bitcast(x_ref[0:ahead, :], u32)
    for cp in chunk_copies(0):
        cp.wait()
    for a in range(1, N_STAGE):
        for cp in chunk_copies(a):
            cp.start()

    def spectrum_ssm(a):
        sgn = jnp.where((lax.broadcasted_iota(jnp.int32, (FB, LANES), 0) & 1) == 0, 1.0, -1.0)
        for cg in range(n_col):
            cs = _lanes(cg)
            kf = lax.dot_general(fwd_ref[...], ssmk_ref[a, cs, :], NT, preferred_element_type=f32)
            for q in range(nfb):
                re, im = slice(2 * q * FB, (2 * q + 1) * FB), slice((2 * q + 1) * FB, (2 * q + 2) * FB)
                cf_ref[q, a, re_blk, cs] = kf[re] - sgn * kprev_ref[im, cs]
                cf_ref[q, a, im_blk, cs] = kf[im] + sgn * kprev_ref[re, cs]
            kprev_ref[:, cs] = kf

    def spectrum_kv(a):
        r0 = pl.multiple_of(a * T, T)
        rows = pl.ds(r0, T)
        before = pl.ds(pl.multiple_of(jnp.maximum(r0 - 16, 0), 16), 16)
        for cg in range(n_col):
            cs = _lanes(cg)
            shift = shift_ref[:, cs].astype(f32)
            prev = jnp.where(a > 0, bk_ref[before, cs].astype(f32)[8:16], 0.0)
            ext = jnp.concatenate([prev, bk_ref[rows, cs].astype(f32)], axis=0)
            ksh = ext[8:8 + T] * shift[0:1]
            for j in range(1, shift.shape[0]):
                ksh = ksh + ext[8 - j:8 - j + T] * shift[j:j + 1]
            kv = (ksh * bv_ref[rows, cs].astype(f32)).astype(bf16)
            kv_ref[rows, cs] = kv
            xf = _dot(fwd_ref[...], kv)
            for q in range(nfb):
                xf_ref[q, xbase + a, :, cs] = xf[2 * q * FB:(2 * q + 2) * FB]

    def chunk(a, c):
        @pl.when(a > 0)
        def _():
            for cp in chunk_copies(a):
                cp.wait()

        slot = a % N_STAGE
        for blk in range(3 * tpp):
            m, t = divmod(blk, tpp)
            if blk == 0:
                wo_rows = pl.ds(pl.multiple_of(a * (pw // 2), pw // 2), pw // 2)
                wo_ref[wo_rows, :] = pltpu.bitcast(stage_ref[slot, 3], u32)
            raw = stage_ref[slot, m, _lanes(t), :]
            w_ref[a * 3 * tpp + blk] = pltpu.bitcast(raw.T, u32)
            y = lax.dot_general(pltpu.bitcast(xh_ref[...], bf16), raw, NT, preferred_element_type=f32)
            rings[m][a * tpp + t, ring_off:ring_off + ahead, :] = y.astype(bf16)
            if blk == 1:
                spectrum_ssm(a)
            if blk == 5:
                spectrum_kv(a)

        @pl.when(a + N_STAGE < n_chunk)
        def _():
            for cp in chunk_copies(a + N_STAGE):
                cp.start()

        @pl.when(a == n_chunk - N_STAGE)
        def _():
            x_tail.start()

        return c

    lax.fori_loop(0, n_chunk, chunk, 0)

    def first_outputs(q, c):
        c0 = cf_ref[q, 0, re_blk], cf_ref[q, 0, im_blk]
        c1 = cf_ref[q, 1, re_blk], cf_ref[q, 1, im_blk]
        x0 = xf_ref[q, xbase, re_blk], xf_ref[q, xbase, im_blk]
        x1 = xf_ref[q, xbase + 1, re_blk], xf_ref[q, xbase + 1, im_blk]
        xf_ref[q, ybase, re_blk], xf_ref[q, ybase, im_blk] = _cmul(*c0, *x0)
        (ar, ai), (br, bi) = _cmul(*c0, *x1), _cmul(*c1, *x0)
        xf_ref[q, ybase + 1, re_blk], xf_ref[q, ybase + 1, im_blk] = ar + br, ai + bi
        return c

    lax.fori_loop(0, nfb, first_outputs, 0)
    x_tail.wait()

    def convolve_spectra(it):
        pair_id, part = it // nfb, it % nfb
        nxt = jnp.minimum(2 * pair_id + 2, n_chunk - 2)
        c_now = cf_ref.at[part]
        x_now = xf_ref.at[part, pl.ds(nxt, n_chunk + 1)]
        y_now = xf_ref.at[part, pl.ds(ybase + 2 * ((pair_id + 1) % 2), 2)]
        for cg in range(n_col):
            for ft in range(FB // 8):
                re, im, cs = slice(ft * 8, ft * 8 + 8), slice(FB + ft * 8, FB + ft * 8 + 8), _lanes(cg)
                y = [None, None]
                hi = x_now[n_chunk, re, cs], x_now[n_chunk, im, cs]
                for dl in range(n_chunk):
                    cc = c_now[dl, re, cs], c_now[dl, im, cs]
                    lo = x_now[n_chunk - 1 - dl, re, cs], x_now[n_chunk - 1 - dl, im, cs]
                    for j, xx in enumerate((lo, hi)):
                        tr, ti = _cmul(*cc, *xx)
                        y[j] = (tr, ti) if y[j] is None else (y[j][0] + tr, y[j][1] + ti)
                    hi = lo
                    if (dl + 1) % 3 == 0 and dl + 1 < n_chunk:
                        y_now[1, im, cs] = y[1][1]
                for j in range(2):
                    y_now[j, re, cs], y_now[j, im, cs] = y[j]

    def gate_and_b(it):
        n = UNROLL * seg
        r0 = pl.multiple_of(it * n, n)
        rows = pl.ds(r0, n)
        inv = inv_ref[pl.ds(pl.multiple_of(r0 % T, n), n), :]
        x = x_ref[rows, :].astype(f32)
        z = jnp.sum(x * vec_ref[1:2, :], axis=1, keepdims=True)
        gate = jnp.broadcast_to(jax.nn.sigmoid(z), (n, LANES))
        out = []
        for cg in range(n_col):
            cs = _lanes(cg)
            yf = xf_ref[:, ybase + (r0 // T) % 4, :, cs].reshape(2 * T, LANES)
            y = _dot(inv, yf.astype(bf16)) + kv_ref[rows, cs].astype(f32) * vec_ref[0:1, cs]
            out.append((1.0 - gate) * (x[:, cs] * y))
        return gate, out

    def step(it, sub, mem, shared):
        s = it * UNROLL + sub
        rd = pl.ds(pl.multiple_of(lax.rem(s * seg + ring_off, ring_rows), seg), seg)
        wr = pl.ds(pl.multiple_of(lax.rem(s * tok, ring_rows), 8), tok)
        x_new = x_ref[pl.ds(pl.multiple_of(ahead + s * tok, 8), tok), :]
        lhs = [jnp.concatenate([mem[n], x_new[:, _lanes(n)].astype(f32)], axis=0).astype(bf16)
               for n in range(n_col)]
        lhs_all = jnp.concatenate(lhs, axis=1)

        half = LANES // 2
        row = lax.broadcasted_iota(jnp.int32, (L, LANES), 0)
        lane = lax.broadcasted_iota(jnp.int32, (L, LANES), 1)
        key = lane & (half - 1)
        is_key = key < L
        allowed = (row < M) | (key >= seg) | (row - M >= key)
        first = lane < half
        first_k = lax.broadcasted_iota(jnp.int32, (half, LANES), 1) < half
        zhalf = jnp.zeros((half, LANES), bf16)
        row_first = lax.broadcasted_iota(jnp.int32, (LANES, LANES), 0) < half
        col_first = lax.broadcasted_iota(jnp.int32, (LANES, LANES), 1) < half

        def weights(p, m, t, n0, n1):
            return pltpu.bitcast(w_ref[(p * 3 + m) * tpp + t, n0 * half:n1 * half, :], bf16)

        def proj(p, m, early=0):
            if early:
                ys = [_dot(lhs_all[:, :early * LANES], weights(p, m, t, 0, early)) for t in range(tpp)]
                for n in range(early, n_col):
                    ys = [y + _dot(lhs[n], weights(p, m, t, n, n + 1)) for t, y in enumerate(ys)]
            out = []
            for t in range(tpp):
                y = ys[t] if early else _dot(lhs_all, weights(p, m, t, 0, n_col))
                rings[m][p * tpp + t, wr, :] = y[M:].astype(bf16)
                out.append(y[0:M])
            return out

        def load(p, m):
            return [rings[m][p * tpp + t, rd, :] for t in range(tpp)]

        def keys(tok3, mem3):
            pad = jnp.zeros((half - L, LANES), f32)
            return [jnp.concatenate([tk, jnp.concatenate([mm, pad], axis=0).astype(bf16)], axis=0)
                    for tk, mm in zip(tok3, mem3)]

        def keys_t(k_tok, k_mem):
            a, mid, b = keys(k_tok, k_mem)
            return jnp.concatenate([a, b], axis=0).T, jnp.concatenate([mid, mid], axis=0).T

        def scores(q_tok, q_mem, kt):
            outer, inner = kt
            zero = jnp.zeros_like(outer)
            kb = (jnp.where(col_first, outer, zero),
                  jnp.where(col_first == row_first, inner, zero),
                  jnp.where(col_first, zero, outer))
            acc = None
            for t in range(tpp):
                y = _dot(jnp.concatenate([q_mem[t], q_tok[t].astype(f32)], axis=0), kb[t])
                acc = y if acc is None else acc + y
            return acc

        def softmax(sc):
            sc = jnp.where(allowed, sc * (Dh ** -0.5), -1000000000.0)
            ninf = -jnp.inf
            m0 = jnp.max(jnp.where(first & is_key, sc, ninf), axis=1, keepdims=True)
            m1 = jnp.max(jnp.where(is_key & ~first, sc, ninf), axis=1, keepdims=True)
            e = jnp.exp(jnp.where(is_key, sc - jnp.where(first, m0, m1), ninf))
            s0 = jnp.sum(jnp.where(first, e, 0.0), axis=1, keepdims=True)
            s1 = jnp.sum(jnp.where(first, 0.0, e), axis=1, keepdims=True)
            return e / jnp.where(first, s0, s1)

        def attend(prob, v_tok, v_mem, p):
            a, mid, b = keys(v_tok, v_mem)
            zero = jnp.zeros_like(mid)
            vb = (jnp.concatenate([a, zhalf], axis=0),
                  jnp.concatenate([jnp.where(first_k, mid, zero), jnp.where(first_k, zero, mid)], axis=0),
                  jnp.concatenate([zhalf, b], axis=0))
            for t in range(tpp):
                att_ref[:, _lanes(p * tpp + t)] = _dot(prob, vb[t])

        accs = [None] * n_col

        def out_proj(p0, p1):
            for n in range(n_col):
                y = _dot(att_ref[:, p0 * pw:p1 * pw],
                         pltpu.bitcast(wo_ref[p0 * pw // 2:p1 * pw // 2, _lanes(n)], bf16))
                accs[n] = y if accs[n] is None else accs[n] + y

        d_kt, d_sc, d_sm, d_pv = 3, 7, 8, 13
        mem_qkv, kt, sc, pr = ({}, {}, {}), {}, {}, {}
        done = 0

        def due(u, d):
            p, r = divmod(u - d, 3)
            return p if r == 0 and 0 <= p < n_pairs else None

        for u in range(3 * n_pairs + d_pv - 2):
            p_kt, p_sc, p_sm, p_pv = due(u, d_kt), due(u, d_sc), due(u, d_sm), due(u, d_pv)
            if p_kt is not None:
                k_tok = load(p_kt, 1)
            if p_sc is not None:
                q_tok = load(p_sc, 0)
            if p_pv is not None:
                v_tok = load(p_pv, 2)
            p, r = divmod(u, 3)
            if p < n_pairs:
                m = (1, 0, 2)[r]
                mem_qkv[m][p] = proj(p, m, early=2 if u == 0 and sub > 0 else 0)
            elif done <= (u - d_pv - 1) // 3:
                out_proj(done, done + 1)
                done += 1
            if p_sc is not None:
                sc[p_sc] = scores(q_tok, mem_qkv[0][p_sc], kt[p_sc])
            if p_pv is not None:
                attend(pr[p_pv], v_tok, mem_qkv[2][p_pv], p_pv)
            if p_kt is not None:
                kt[p_kt] = keys_t(k_tok, mem_qkv[1][p_kt])
            if p_sm is not None:
                pr[p_sm] = softmax(sc[p_sm])
            if sub == 0 and u == 2:
                shared.extend(gate_and_b(it))
            if sub == 0 and u == 3:
                convolve_spectra(it)
        out_proj(done, n_pairs)

        gate, gated_b = shared
        mine = slice(sub * seg, (sub + 1) * seg)
        rows = pl.ds(pl.multiple_of(s * seg, seg), seg)
        for n in range(n_col):
            res = gate[mine] * accs[n][M:L] + gated_b[n][mine]
            o_ref[rows, _lanes(n)] = res.astype(o_ref.dtype)
        return [acc[0:M] for acc in accs]

    def steps(it, mem):
        shared = []
        for sub in range(UNROLL):
            mem = step(it, sub, mem, shared)
        return mem

    def steps_and_copy(j, mem):
        per = OUT_STEPS // UNROLL
        mem = steps(j, mem) if per == 1 else lax.fori_loop(j * per, (j + 1) * per, steps, mem)
        rows = pl.ds(pl.multiple_of(j * OUT_STEPS * seg, OUT_STEPS * seg), OUT_STEPS * seg)
        pltpu.make_async_copy(o_ref.at[rows, :], o_hbm.at[rows, :], o_sem).start()
        return mem

    mem0 = [mem0_ref[:, _lanes(n)].astype(f32) for n in range(n_col)]
    lax.fori_loop(0, n_seg // OUT_STEPS, steps_and_copy, mem0)
    pltpu.make_async_copy(o_ref, o_hbm, o_sem).wait()


@functools.partial(jax.jit, static_argnames=("A_seg_len",))
def pallas_gated_mix__memory_aug_recurrent_mem_tr__ssm_conv_h3__prompt_kernel(
    A_x: jax.Array,
    A_mem0: jax.Array,
    A_Wq: jax.Array,
    A_Wk: jax.Array,
    A_Wv: jax.Array,
    A_Wo: jax.Array,
    A_seg_len: int,
    B_q: jax.Array,
    B_k: jax.Array,
    B_v: jax.Array,
    B_shift_k: jax.Array,
    B_ssm_k: jax.Array,
    B_ssm_D: jax.Array,
    gate_w: jax.Array,
):
    del B_q
    B, S, D = A_x.shape
    H, Dh = A_Wq.shape[1], A_Wq.shape[2]
    M = A_mem0.shape[1]
    seg = int(A_seg_len)
    E = H * Dh
    n_chunk = S // T
    assert (B, M, seg) == (1, 8, 32) and S % (2 * T) == 0 and n_chunk > N_STAGE
    assert (H, 2 * Dh) == (2 * n_chunk, 3 * LANES)
    assert D % LANES == 0 and B_shift_k.shape[1] <= 9
    ahead = (S // seg) * M
    tok = seg - M
    ring_off = next(o for o in range(seg, seg * (tok + 1), seg) if (ahead + o) % tok == 0)
    ring_rows = pl.cdiv(ahead + ring_off, math.lcm(tok, seg)) * math.lcm(tok, seg)

    def head_major(w):
        return jnp.transpose(w, (1, 2, 0)).reshape(E, D)

    fwd, inv = _dft_matrices()
    hbm = pl.BlockSpec(memory_space=pl.ANY)
    vmem = pl.BlockSpec(memory_space=pltpu.VMEM)
    ring = pltpu.VMEM((E // LANES, ring_rows, LANES), bf16)
    out = pl.pallas_call(
        functools.partial(_kernel, S=S, D=D, H=H, Dh=Dh, M=M, seg=seg, ahead=ahead,
                          ring_rows=ring_rows, ring_off=ring_off),
        in_specs=[hbm, vmem, hbm, hbm, hbm, hbm, hbm, hbm, vmem, hbm, vmem, vmem, vmem, vmem],
        out_specs=hbm,
        out_shape=jax.ShapeDtypeStruct((S, D), A_x.dtype),
        scratch_shapes=[
            pltpu.VMEM((S, D), bf16),
            pltpu.VMEM((S, D), bf16),
            pltpu.VMEM((S, D), bf16),
            pltpu.VMEM((n_chunk, D, T), bf16),
            pltpu.VMEM((N_STAGE, 4, 2 * Dh, D), bf16),
            pltpu.VMEM((3 * E // LANES, D // 2, LANES), u32),
            pltpu.VMEM((E // 2, D), u32),
            pltpu.VMEM((ahead // 2, D), u32),
            ring, ring, ring,
            pltpu.VMEM((S, D), bf16),
            pltpu.VMEM((T // FB, 2 * n_chunk + 3, 2 * FB, D), f32),
            pltpu.VMEM((T // FB, n_chunk, 2 * FB, D), f32),
            pltpu.VMEM((2 * T, D), f32),
            pltpu.VMEM((M + seg, E), f32),
            pltpu.VMEM((S, D), A_x.dtype),
            pltpu.VMEM((2, D), f32),
            pltpu.SemaphoreType.DMA((2,)),
            pltpu.SemaphoreType.DMA((4, n_chunk)),
            pltpu.SemaphoreType.DMA((3, n_chunk)),
            pltpu.SemaphoreType.DMA(()),
        ],
        compiler_params=pltpu.CompilerParams(
            vmem_limit_bytes=120 * 1024 * 1024,
            disable_bounds_checks=True,
        ),
    )(
        A_x.reshape(S, D), A_mem0.reshape(M, D),
        head_major(A_Wq), head_major(A_Wk), head_major(A_Wv), A_Wo.reshape(E, D),
        B_k.reshape(S, D), B_v.reshape(S, D), B_shift_k.T, B_ssm_k, B_ssm_D, gate_w,
        fwd, inv,
    )
    return out.reshape(B, S, D)
```

```python
import functools
import math

import jax
import jax.numpy as jnp
import numpy as np
from jax import lax
from jax.experimental import pallas as pl
from jax.experimental.pallas import tpu as pltpu

f32 = jnp.float32
u32 = jnp.uint32
bf16 = jnp.bfloat16
NT = (((1,), (1,)), ((), ()))
LANES = 128
T = 128
N_STAGE = 3
UNROLL = 2
FB = 16 * UNROLL
OUT_STEPS = 2


def _dft_matrices():
    theta = 2.0 * np.pi * (np.arange(T, dtype=np.float64) + 0.5) / (2 * T)
    ang = theta[:, None] * np.arange(T, dtype=np.float64)[None, :]
    fwd = np.stack([np.cos(ang).reshape(-1, FB, T), -np.sin(ang).reshape(-1, FB, T)], axis=1)
    fwd = fwd.reshape(2 * T, T)
    return fwd.astype(bf16), (fwd.T / T).astype(bf16)


def _dot(a, b):
    return jnp.dot(a, b, preferred_element_type=f32)


def _lanes(i):
    return slice(i * LANES, (i + 1) * LANES)


def _cmul(ar, ai, br, bi):
    return ar * br - ai * bi, ar * bi + ai * br


def _kernel(
    x_hbm, mem0_hbm, wq_hbm, wk_hbm, wv_hbm, wo_hbm, bk_hbm, bv_hbm, shift_hbm,
    ssmk_hbm, ssmd_hbm, gw_hbm, fwd_hbm, inv_hbm,
    o_hbm,
    x_ref, bk_ref, bv_ref, ssmk_ref, stage_ref, w_ref, wo_ref, xh_ref, q_ring, k_ring, v_ring,
    kv_ref, xf_ref, cf_ref, kprev_ref, att_ref, o_ref, fwd_ref, inv_ref,
    vec_ref, mem0_ref, shift_ref, ssmd_ref, gw_ref,
    s_sem, x_sem, w_sem, c_sem, o_sem,
    *, S, D, H, Dh, M, seg, ahead, ring_rows, ring_off,
):
    L = M + seg
    n_seg = S // seg
    n_pairs = H // 2
    pw = 2 * Dh
    tpp = pw // LANES
    n_col = D // LANES
    n_chunk = S // T
    nfb = T // FB
    xbase = n_chunk - 1
    ybase = xbase + n_chunk
    tok = seg - M
    rings = (q_ring, k_ring, v_ring)
    w_hbm = (wq_hbm, wk_hbm, wv_hbm, wo_hbm)
    re_blk, im_blk = slice(0, FB), slice(FB, 2 * FB)

    def chunk_copies(a):
        wrows = pl.ds(pl.multiple_of(a * pw, pw), pw)
        trows = pl.ds(pl.multiple_of(a * T, T), T)
        return [
            pltpu.make_async_copy(w_hbm[m].at[wrows, :], stage_ref.at[a % N_STAGE, m], w_sem.at[m, a])
            for m in range(4)
        ] + [
            pltpu.make_async_copy(bk_hbm.at[trows, :], bk_ref.at[trows, :], c_sem.at[0, a]),
            pltpu.make_async_copy(bv_hbm.at[trows, :], bv_ref.at[trows, :], c_sem.at[1, a]),
            pltpu.make_async_copy(ssmk_hbm.at[:, trows], ssmk_ref.at[a], c_sem.at[2, a]),
        ]

    x_head = pltpu.make_async_copy(x_hbm.at[0:ahead, :], x_ref.at[0:ahead, :], x_sem.at[0])
    x_tail = pltpu.make_async_copy(x_hbm.at[ahead:S, :], x_ref.at[ahead:S, :], x_sem.at[1])
    small = [
        pltpu.make_async_copy(src, dst, s_sem.at[i])
        for i, (src, dst) in enumerate([
            (mem0_hbm, mem0_ref), (shift_hbm, shift_ref), (ssmd_hbm, ssmd_ref),
            (gw_hbm, gw_ref), (fwd_hbm, fwd_ref), (inv_hbm, inv_ref)])
    ]
    for cp in small + [x_head] + chunk_copies(0):
        cp.start()

    def zero(a, c):
        for q in range(nfb):
            xf_ref[q, a] = jnp.zeros(xf_ref.shape[2:], f32)
        return c

    lax.fori_loop(0, xbase, zero, 0)
    kprev_ref[...] = jnp.zeros(kprev_ref.shape, f32)
    for cp in small:
        cp.wait()
    vec_ref[0:1, :] = ssmd_ref[...].astype(f32).reshape(1, D)
    vec_ref[1:2, :] = gw_ref[...].astype(f32).reshape(1, D)
    x_head.wait()
    xh_ref[...] = pltpu.bitcast(x_ref[0:ahead, :], u32)
    for cp in chunk_copies(0):
        cp.wait()
    for a in range(1, N_STAGE):
        for cp in chunk_copies(a):
            cp.start()

    def spectrum_ssm(a):
        sgn = jnp.where((lax.broadcasted_iota(jnp.int32, (FB, LANES), 0) & 1) == 0, 1.0, -1.0)
        for cg in range(n_col):
            cs = _lanes(cg)
            kf = lax.dot_general(fwd_ref[...], ssmk_ref[a, cs, :], NT, preferred_element_type=f32)
            for q in range(nfb):
                re, im = slice(2 * q * FB, (2 * q + 1) * FB), slice((2 * q + 1) * FB, (2 * q + 2) * FB)
                cf_ref[q, a, re_blk, cs] = kf[re] - sgn * kprev_ref[im, cs]
                cf_ref[q, a, im_blk, cs] = kf[im] + sgn * kprev_ref[re, cs]
            kprev_ref[:, cs] = kf

    def spectrum_kv(a):
        r0 = pl.multiple_of(a * T, T)
        rows = pl.ds(r0, T)
        before = pl.ds(pl.multiple_of(jnp.maximum(r0 - 16, 0), 16), 16)
        for cg in range(n_col):
            cs = _lanes(cg)
            shift = shift_ref[:, cs].astype(f32)
            prev = jnp.where(a > 0, bk_ref[before, cs].astype(f32)[8:16], 0.0)
            ext = jnp.concatenate([prev, bk_ref[rows, cs].astype(f32)], axis=0)
            ksh = ext[8:8 + T] * shift[0:1]
            for j in range(1, shift.shape[0]):
                ksh = ksh + ext[8 - j:8 - j + T] * shift[j:j + 1]
            kv = (ksh * bv_ref[rows, cs].astype(f32)).astype(bf16)
            kv_ref[rows, cs] = kv
            xf = _dot(fwd_ref[...], kv)
            for q in range(nfb):
                xf_ref[q, xbase + a, :, cs] = xf[2 * q * FB:(2 * q + 2) * FB]

    def chunk(a, c):
        @pl.when(a > 0)
        def _():
            for cp in chunk_copies(a):
                cp.wait()

        slot = a % N_STAGE
        for blk in range(3 * tpp):
            m, t = divmod(blk, tpp)
            if blk == 0:
                wo_rows = pl.ds(pl.multiple_of(a * (pw // 2), pw // 2), pw // 2)
                wo_ref[wo_rows, :] = pltpu.bitcast(stage_ref[slot, 3], u32)
            raw = stage_ref[slot, m, _lanes(t), :]
            w_ref[a * 3 * tpp + blk] = pltpu.bitcast(raw.T, u32)
            y = lax.dot_general(pltpu.bitcast(xh_ref[...], bf16), raw, NT, preferred_element_type=f32)
            rings[m][a * tpp + t, ring_off:ring_off + ahead, :] = y.astype(bf16)
            if blk == 1:
                spectrum_ssm(a)
            if blk == 5:
                spectrum_kv(a)

        @pl.when(a + N_STAGE < n_chunk)
        def _():
            for cp in chunk_copies(a + N_STAGE):
                cp.start()

        @pl.when(a == n_chunk - N_STAGE)
        def _():
            x_tail.start()

        return c

    lax.fori_loop(0, n_chunk, chunk, 0)

    def first_outputs(q, c):
        c0 = cf_ref[q, 0, re_blk], cf_ref[q, 0, im_blk]
        c1 = cf_ref[q, 1, re_blk], cf_ref[q, 1, im_blk]
        x0 = xf_ref[q, xbase, re_blk], xf_ref[q, xbase, im_blk]
        x1 = xf_ref[q, xbase + 1, re_blk], xf_ref[q, xbase + 1, im_blk]
        xf_ref[q, ybase, re_blk], xf_ref[q, ybase, im_blk] = _cmul(*c0, *x0)
        (ar, ai), (br, bi) = _cmul(*c0, *x1), _cmul(*c1, *x0)
        xf_ref[q, ybase + 1, re_blk], xf_ref[q, ybase + 1, im_blk] = ar + br, ai + bi
        return c

    lax.fori_loop(0, nfb, first_outputs, 0)
    x_tail.wait()

    def convolve_spectra(it):
        pair_id, part = it // nfb, it % nfb
        nxt = jnp.minimum(2 * pair_id + 2, n_chunk - 2)
        c_now = cf_ref.at[part]
        x_now = xf_ref.at[part, pl.ds(nxt, n_chunk + 1)]
        y_now = xf_ref.at[part, pl.ds(ybase + 2 * ((pair_id + 1) % 2), 2)]
        for cg in range(n_col):
            for ft in range(FB // 8):
                re, im, cs = slice(ft * 8, ft * 8 + 8), slice(FB + ft * 8, FB + ft * 8 + 8), _lanes(cg)
                y = [None, None]
                hi = x_now[n_chunk, re, cs], x_now[n_chunk, im, cs]
                for dl in range(n_chunk):
                    cc = c_now[dl, re, cs], c_now[dl, im, cs]
                    lo = x_now[n_chunk - 1 - dl, re, cs], x_now[n_chunk - 1 - dl, im, cs]
                    for j, xx in enumerate((lo, hi)):
                        tr, ti = _cmul(*cc, *xx)
                        y[j] = (tr, ti) if y[j] is None else (y[j][0] + tr, y[j][1] + ti)
                    hi = lo
                    if (dl + 1) % 3 == 0 and dl + 1 < n_chunk:
                        y_now[1, im, cs] = y[1][1]
                for j in range(2):
                    y_now[j, re, cs], y_now[j, im, cs] = y[j]

    def gate_and_b(it):
        n = UNROLL * seg
        r0 = pl.multiple_of(it * n, n)
        rows = pl.ds(r0, n)
        inv = inv_ref[pl.ds(pl.multiple_of(r0 % T, n), n), :]
        x = x_ref[rows, :].astype(f32)
        z = jnp.sum(x * vec_ref[1:2, :], axis=1, keepdims=True)
        gate = jnp.broadcast_to(jax.nn.sigmoid(z), (n, LANES))
        out = []
        for cg in range(n_col):
            cs = _lanes(cg)
            yf = xf_ref[:, ybase + (r0 // T) % 4, :, cs].reshape(2 * T, LANES)
            y = _dot(inv, yf.astype(bf16)) + kv_ref[rows, cs].astype(f32) * vec_ref[0:1, cs]
            out.append((1.0 - gate) * (x[:, cs] * y))
        return gate, out

    def step(it, sub, mem, shared):
        s = it * UNROLL + sub
        rd = pl.ds(pl.multiple_of(lax.rem(s * seg + ring_off, ring_rows), seg), seg)
        wr = pl.ds(pl.multiple_of(lax.rem(s * tok, ring_rows), 8), tok)
        x_new = x_ref[pl.ds(pl.multiple_of(ahead + s * tok, 8), tok), :]
        lhs = [jnp.concatenate([mem[n], x_new[:, _lanes(n)].astype(f32)], axis=0).astype(bf16)
               for n in range(n_col)]
        lhs_all = jnp.concatenate(lhs, axis=1)

        half = LANES // 2
        row = lax.broadcasted_iota(jnp.int32, (L, LANES), 0)
        lane = lax.broadcasted_iota(jnp.int32, (L, LANES), 1)
        key = lane & (half - 1)
        is_key = key < L
        allowed = (row < M) | (key >= seg) | (row - M >= key)
        first = lane < half
        first_k = lax.broadcasted_iota(jnp.int32, (half, LANES), 1) < half
        zhalf = jnp.zeros((half, LANES), bf16)
        row_first = lax.broadcasted_iota(jnp.int32, (LANES, LANES), 0) < half
        col_first = lax.broadcasted_iota(jnp.int32, (LANES, LANES), 1) < half

        def weights(p, m, t, n0, n1):
            return pltpu.bitcast(w_ref[(p * 3 + m) * tpp + t, n0 * half:n1 * half, :], bf16)

        def proj(p, m, early=0):
            if early:
                ys = [_dot(lhs_all[:, :early * LANES], weights(p, m, t, 0, early)) for t in range(tpp)]
                for n in range(early, n_col):
                    ys = [y + _dot(lhs[n], weights(p, m, t, n, n + 1)) for t, y in enumerate(ys)]
            out = []
            for t in range(tpp):
                y = ys[t] if early else _dot(lhs_all, weights(p, m, t, 0, n_col))
                rings[m][p * tpp + t, wr, :] = y[M:].astype(bf16)
                out.append(y[0:M])
            return out

        def load(p, m):
            return [rings[m][p * tpp + t, rd, :] for t in range(tpp)]

        def keys(tok3, mem3):
            pad = jnp.zeros((half - L, LANES), f32)
            return [jnp.concatenate([tk, jnp.concatenate([mm, pad], axis=0).astype(bf16)], axis=0)
                    for tk, mm in zip(tok3, mem3)]

        def keys_t(k_tok, k_mem):
            a, mid, b = keys(k_tok, k_mem)
            return jnp.concatenate([a, b], axis=0).T, jnp.concatenate([mid, mid], axis=0).T

        def scores(q_tok, q_mem, kt):
            outer, inner = kt
            zero = jnp.zeros_like(outer)
            kb = (jnp.where(col_first, outer, zero),
                  jnp.where(col_first == row_first, inner, zero),
                  jnp.where(col_first, zero, outer))
            acc = None
            for t in range(tpp):
                y = _dot(jnp.concatenate([q_mem[t], q_tok[t].astype(f32)], axis=0), kb[t])
                acc = y if acc is None else acc + y
            return acc

        def softmax(sc):
            sc = jnp.where(allowed, sc * (Dh ** -0.5), -1000000000.0)
            ninf = -jnp.inf
            m0 = jnp.max(jnp.where(first & is_key, sc, ninf), axis=1, keepdims=True)
            m1 = jnp.max(jnp.where(is_key & ~first, sc, ninf), axis=1, keepdims=True)
            e = jnp.exp(jnp.where(is_key, sc - jnp.where(first, m0, m1), ninf))
            s0 = jnp.sum(jnp.where(first, e, 0.0), axis=1, keepdims=True)
            s1 = jnp.sum(jnp.where(first, 0.0, e), axis=1, keepdims=True)
            return e / jnp.where(first, s0, s1)

        def attend(prob, v_tok, v_mem, p):
            a, mid, b = keys(v_tok, v_mem)
            zero = jnp.zeros_like(mid)
            vb = (jnp.concatenate([a, zhalf], axis=0),
                  jnp.concatenate([jnp.where(first_k, mid, zero), jnp.where(first_k, zero, mid)], axis=0),
                  jnp.concatenate([zhalf, b], axis=0))
            for t in range(tpp):
                att_ref[:, _lanes(p * tpp + t)] = _dot(prob, vb[t])

        accs = [None] * n_col

        def out_proj(p0, p1):
            for n in range(n_col):
                y = _dot(att_ref[:, p0 * pw:p1 * pw],
                         pltpu.bitcast(wo_ref[p0 * pw // 2:p1 * pw // 2, _lanes(n)], bf16))
                accs[n] = y if accs[n] is None else accs[n] + y

        d_kt, d_sc, d_sm, d_pv = 3, 7, 8, 13
        mem_qkv, kt, sc, pr = ({}, {}, {}), {}, {}, {}
        done = 0

        def due(u, d):
            p, r = divmod(u - d, 3)
            return p if r == 0 and 0 <= p < n_pairs else None

        for u in range(3 * n_pairs + d_pv - 2):
            p_kt, p_sc, p_sm, p_pv = due(u, d_kt), due(u, d_sc), due(u, d_sm), due(u, d_pv)
            if p_kt is not None:
                k_tok = load(p_kt, 1)
            if p_sc is not None:
                q_tok = load(p_sc, 0)
            if p_pv is not None:
                v_tok = load(p_pv, 2)
            p, r = divmod(u, 3)
            if p < n_pairs:
                m = (1, 0, 2)[r]
                mem_qkv[m][p] = proj(p, m, early=2 if u == 0 and sub > 0 else 0)
            elif done <= (u - d_pv - 1) // 3:
                out_proj(done, done + 1)
                done += 1
            if p_sc is not None:
                sc[p_sc] = scores(q_tok, mem_qkv[0][p_sc], kt[p_sc])
            if p_pv is not None:
                attend(pr[p_pv], v_tok, mem_qkv[2][p_pv], p_pv)
            if p_kt is not None:
                kt[p_kt] = keys_t(k_tok, mem_qkv[1][p_kt])
            if p_sm is not None:
                pr[p_sm] = softmax(sc[p_sm])
            if sub == 0 and u == 2:
                shared.extend(gate_and_b(it))
            if sub == 0 and u == 3:
                convolve_spectra(it)
        out_proj(done, n_pairs)

        gate, gated_b = shared
        mine = slice(sub * seg, (sub + 1) * seg)
        rows = pl.ds(pl.multiple_of(s * seg, seg), seg)
        for n in range(n_col):
            res = gate[mine] * accs[n][M:L] + gated_b[n][mine]
            o_ref[rows, _lanes(n)] = res.astype(o_ref.dtype)
        return [acc[0:M] for acc in accs]

    def steps(it, mem):
        shared = []
        for sub in range(UNROLL):
            mem = step(it, sub, mem, shared)
        return mem

    def steps_and_copy(j, mem):
        per = OUT_STEPS // UNROLL
        mem = steps(j, mem) if per == 1 else lax.fori_loop(j * per, (j + 1) * per, steps, mem)
        rows = pl.ds(pl.multiple_of(j * OUT_STEPS * seg, OUT_STEPS * seg), OUT_STEPS * seg)
        pltpu.make_async_copy(o_ref.at[rows, :], o_hbm.at[rows, :], o_sem).start()
        return mem

    mem0 = [mem0_ref[:, _lanes(n)].astype(f32) for n in range(n_col)]
    lax.fori_loop(0, n_seg // OUT_STEPS, steps_and_copy, mem0)
    pltpu.make_async_copy(o_ref, o_hbm, o_sem).wait()


@functools.partial(jax.jit, static_argnames=("A_seg_len",))
def pallas_gated_mix__memory_aug_recurrent_mem_tr__ssm_conv_h3__prompt_kernel(
    A_x: jax.Array,
    A_mem0: jax.Array,
    A_Wq: jax.Array,
    A_Wk: jax.Array,
    A_Wv: jax.Array,
    A_Wo: jax.Array,
    A_seg_len: int,
    B_q: jax.Array,
    B_k: jax.Array,
    B_v: jax.Array,
    B_shift_k: jax.Array,
    B_ssm_k: jax.Array,
    B_ssm_D: jax.Array,
    gate_w: jax.Array,
):
    del B_q
    B, S, D = A_x.shape
    H, Dh = A_Wq.shape[1], A_Wq.shape[2]
    M = A_mem0.shape[1]
    seg = int(A_seg_len)
    E = H * Dh
    n_chunk = S // T
    assert (B, M, seg) == (1, 8, 32) and S % (2 * T) == 0 and n_chunk > N_STAGE
    assert (H, 2 * Dh) == (2 * n_chunk, 3 * LANES)
    assert D % LANES == 0 and B_shift_k.shape[1] <= 9
    ahead = (S // seg) * M
    tok = seg - M
    ring_off = next(o for o in range(seg, seg * (tok + 1), seg) if (ahead + o) % tok == 0)
    ring_rows = pl.cdiv(ahead + ring_off, math.lcm(tok, seg)) * math.lcm(tok, seg)

    def head_major(w):
        return jnp.transpose(w, (1, 2, 0)).reshape(E, D)

    fwd, inv = _dft_matrices()
    hbm = pl.BlockSpec(memory_space=pl.ANY)
    ring = pltpu.VMEM((E // LANES, ring_rows, LANES), bf16)
    out = pl.pallas_call(
        functools.partial(_kernel, S=S, D=D, H=H, Dh=Dh, M=M, seg=seg, ahead=ahead,
                          ring_rows=ring_rows, ring_off=ring_off),
        in_specs=[hbm] * 14,
        out_specs=hbm,
        out_shape=jax.ShapeDtypeStruct((S, D), A_x.dtype),
        scratch_shapes=[
            pltpu.VMEM((S, D), bf16),
            pltpu.VMEM((S, D), bf16),
            pltpu.VMEM((S, D), bf16),
            pltpu.VMEM((n_chunk, D, T), bf16),
            pltpu.VMEM((N_STAGE, 4, 2 * Dh, D), bf16),
            pltpu.VMEM((3 * E // LANES, D // 2, LANES), u32),
            pltpu.VMEM((E // 2, D), u32),
            pltpu.VMEM((ahead // 2, D), u32),
            ring, ring, ring,
            pltpu.VMEM((S, D), bf16),
            pltpu.VMEM((T // FB, 2 * n_chunk + 3, 2 * FB, D), f32),
            pltpu.VMEM((T // FB, n_chunk, 2 * FB, D), f32),
            pltpu.VMEM((2 * T, D), f32),
            pltpu.VMEM((M + seg, E), f32),
            pltpu.VMEM((S, D), A_x.dtype),
            pltpu.VMEM((2 * T, T), bf16),
            pltpu.VMEM((T, 2 * T), bf16),
            pltpu.VMEM((2, D), f32),
            pltpu.VMEM((M, D), bf16),
            pltpu.VMEM((B_shift_k.shape[1], D), bf16),
            pltpu.VMEM((D,), bf16),
            pltpu.VMEM((D,), bf16),
            pltpu.SemaphoreType.DMA((6,)),
            pltpu.SemaphoreType.DMA((2,)),
            pltpu.SemaphoreType.DMA((4, n_chunk)),
            pltpu.SemaphoreType.DMA((3, n_chunk)),
            pltpu.SemaphoreType.DMA(()),
        ],
        compiler_params=pltpu.CompilerParams(
            vmem_limit_bytes=120 * 1024 * 1024,
            disable_bounds_checks=True,
        ),
    )(
        A_x.reshape(S, D), A_mem0.reshape(M, D),
        head_major(A_Wq), head_major(A_Wk), head_major(A_Wv), A_Wo.reshape(E, D),
        B_k.reshape(S, D), B_v.reshape(S, D), B_shift_k.T, B_ssm_k, B_ssm_D, gate_w,
        fwd, inv,
    )
    return out.reshape(B, S, D)
```
